```python
import jax
import jax.numpy as jnp

def _softmax(x, axis=-1):
    return jax.nn.softmax(x, axis=axis)
def _gelu(x):
    return jax.nn.gelu(x, approximate=True)
def _silu(x):
    return jax.nn.silu(x)
def _sigmoid(x):
    return jax.nn.sigmoid(x)
def _layernorm(x, axis=-1, eps=1e-5):
    m = jnp.mean(x, axis=axis, keepdims=True)
    v = jnp.var(x, axis=axis, keepdims=True)
    return (x - m) / jnp.sqrt(v + eps)
def _scatter_add(tgt, idx, src, axis=0):
    return tgt.at[idx].add(src)
def _segment_sum(src, seg, n):
    return jax.ops.segment_sum(src, seg, n)
class _Rng:
    def __init__(self, key):
        self._k = key
    def _next(self):
        self._k, sub = jax.random.split(self._k)
        return sub
    def normal(self, shape):
        return jax.random.normal(self._next(), shape, dtype=jnp.bfloat16)
    def randint(self, lo, hi, shape):
        return jax.random.randint(self._next(), shape, lo, hi, dtype=jnp.int32)
    def uniform(self, shape, lo=0.0, hi=1.0):
        return jax.random.uniform(self._next(), shape, jnp.bfloat16, lo, hi)
    def permutation(self, n):
        return jax.random.permutation(self._next(), n)


kernel_name = 'recurrent_scan__compressed_kv_cla__dense_activation_silu__decode'

def setup_inputs():
    _rng = _Rng(jax.random.key(int.from_bytes(__import__("os").urandom(4), "little")))
    _w = (lambda a: (lambda t: t.astype(jnp.bfloat16) if jnp.issubdtype(t.dtype, jnp.floating) else t)(jnp.asarray(a)))
    def _A_setup():
        B, H, Sq, Sk, D, M = 1, 32, 1, 32768, 128, 512
        Dc = 4 * D
        return {
            "x": _w((lambda *s: _rng.normal(s) * 0.05)(B, Sq, M)),
            "c_kv": _w((lambda *s: _rng.normal(s) * 0.05)(B, Sk, Dc)),
            "w_q": _w((lambda *s: _rng.normal(s) * 0.05)(M, H, D) * (M ** -0.5)),
            "w_uk": _w((lambda *s: _rng.normal(s) * 0.05)(Dc, H, D) * (Dc ** -0.5)),
            "w_uv": _w((lambda *s: _rng.normal(s) * 0.05)(Dc, H, D) * (Dc ** -0.5)),
            "w_o": _w((lambda *s: _rng.normal(s) * 0.05)(H, D, M) * ((H * D) ** -0.5)),
        }
    _A_in = _A_setup()

    def _B_setup():
        B, S, D, F = 1, 1, 512, 1376
        return {
            "x": _w((lambda *s: _rng.normal(s) * 0.05)(B, S, D)),
            "w1": _w((lambda *s: _rng.normal(s) * 0.05)(D, F) * (D ** -0.5)),
            "w2": _w((lambda *s: _rng.normal(s) * 0.05)(F, D) * (F ** -0.5)),
        }
    _B_in = _B_setup()

    return {
        "A_x": _A_in["x"],
        "A_c_kv": _A_in["c_kv"],
        "A_w_q": _A_in["w_q"],
        "A_w_uk": _A_in["w_uk"],
        "A_w_uv": _A_in["w_uv"],
        "A_w_o": _A_in["w_o"],
        "B_x": _B_in["x"],
        "B_w1": _B_in["w1"],
        "B_w2": _B_in["w2"],
    }

def reference(A_x, A_c_kv, A_w_q, A_w_uk, A_w_uv, A_w_o, B_x, B_w1, B_w2):
    def _A_ref(x, c_kv, w_q, w_uk, w_uv, w_o):
        B, Sq, M = x.shape[0], x.shape[1], x.shape[2]
        Sk = c_kv.shape[1]
        H, D = w_q.shape[1], w_q.shape[2]
        q = jnp.einsum("bqm,mhd->bhqd", x, w_q)
        k = jnp.einsum("bkc,chd->bhkd", c_kv, w_uk)
        v = jnp.einsum("bkc,chd->bhkd", c_kv, w_uv)
        scores = jnp.einsum("bhqd,bhkd->bhqk", q, k) * (D ** -0.5)
        off = Sk - Sq
        qi = jnp.arange(Sq)[:, None]
        kj = jnp.arange(Sk)[None, :]
        cmask = kj <= (qi + off)
        scores = jnp.where(cmask[None, None], scores, -1e9)
        p = _softmax(scores, axis=-1)
        ctx = jnp.einsum("bhqk,bhkd->bhqd", p, v)
        return jnp.einsum("bhqd,hdm->bqm", ctx, w_o)

    def _B_ref(x, w1, w2):
        h = jnp.einsum("bsd,df->bsf", x, w1)
        h = _silu(h)
        out = jnp.einsum("bsf,fd->bsd", h, w2)
        return out

    x = A_x
    xn = _layernorm(x, axis=-1)
    s = _A_ref(xn, A_c_kv, A_w_q, A_w_uk, A_w_uv, A_w_o)
    g = _silu(_B_ref(xn, B_w1, B_w2))
    return x + s * g
```

```python
import jax
import jax.numpy as jnp
from jax import lax
import jax.experimental.pallas as pl
import jax.experimental.pallas.tpu as pltpu

_NT = (((1,), (1,)), ((), ()))
_F32 = jnp.float32
_BF16 = jnp.bfloat16


def _silu(v):
    return v * (1.0 / (1.0 + jnp.exp(-v)))


@jax.jit
def pallas_recurrent_scan__compressed_kv_cla__dense_activation_silu__decode_kernel(
    A_x: jax.Array,
    A_c_kv: jax.Array,
    A_w_q: jax.Array,
    A_w_uk: jax.Array,
    A_w_uv: jax.Array,
    A_w_o: jax.Array,
    B_x: jax.Array,
    B_w1: jax.Array,
    B_w2: jax.Array,
):
    del B_x
    B, Sq, M = A_x.shape
    _, S, DC = A_c_kv.shape
    _, H, D = A_w_q.shape
    F = B_w1.shape[1]
    assert B == 1 and Sq == 1 and D == 128 and H == 32 and M == 512 and DC == 512

    T = 2048
    KV_CHUNKS = (8192, 8192, 8192, 8192)
    assert sum(KV_CHUNKS) == S
    NB = 4
    LW = 128 * H
    PIECE = 512

    ckv2 = A_c_kv.reshape(S, DC)
    wq2 = A_w_q.reshape(M * H, D)
    wuk2 = A_w_uk.reshape(DC * H, D)
    wuv2 = A_w_uv.reshape(DC * H, D)
    wo2 = A_w_o.reshape(H * D, M)
    w1t = B_w1.T

    WO_SPLIT = (0, 24 * D, 30 * D, 32 * D)

    def kernel(x_hbm, ckv_hbm, wq_hbm, wuk_hbm, wuv_hbm, wo_hbm, w1_hbm, w2_hbm,
               o_ref,
               x_v, ckv_v, wq_v, wuk_v, wuv_v, wo_v, w1_v, w2_v, e_v, xn_v, lhs_v, sems):
        copies = []

        def add(src, dst):
            copies.append(pltpu.make_async_copy(src, dst, sems.at[len(copies)]))
            return copies[-1]

        c_x = add(x_hbm, x_v)
        c_w1 = add(w1_hbm, w1_v)
        c_w2 = add(w2_hbm, w2_v)
        c_wq = add(wq_hbm, wq_v)
        c_wuk = add(wuk_hbm, wuk_v)
        c_kv = []
        off = 0
        for n in KV_CHUNKS:
            c_kv.append(add(ckv_hbm.at[pl.ds(off, n)], ckv_v.at[pl.ds(off, n)]))
            off += n
        c_wuv = add(wuv_hbm, wuv_v)
        c_wo = []
        for a, b in zip(WO_SPLIT[:-1], WO_SPLIT[1:]):
            c_wo.append(add(wo_hbm.at[pl.ds(a, b - a)], wo_v.at[pl.ds(a, b - a)]))

        c_x.start()
        c_w1.start()
        c_w2.start()
        c_wq.start()

        for n in range(LW // PIECE):
            row = lax.broadcasted_iota(jnp.int32, (128, PIECE), 0)
            col = lax.broadcasted_iota(jnp.int32, (128, PIECE), 1) + n * PIECE
            e_v[:, n * PIECE:(n + 1) * PIECE] = jnp.where(
                row == (col >> 5), 1.0, 0.0).astype(_BF16)

        def head_mask(rows):
            r = lax.broadcasted_iota(jnp.int32, (rows, PIECE), 0)
            c = lax.broadcasted_iota(jnp.int32, (rows, PIECE), 1)
            return (r & (H - 1)) == (c & (H - 1))

        def diag_contract(a, w_ref):
            a4 = jnp.concatenate(
                [a[:, b * 128:(b + 1) * 128] for b in range(NB)], axis=0)
            mask = head_mask(NB * H)
            out = jnp.zeros((H, D), _F32)
            for n in range(LW // PIECE):
                r = jnp.dot(a4, e_v[:, n * PIECE:(n + 1) * PIECE],
                            preferred_element_type=_F32)
                xm = jnp.where(mask, r, 0.0).astype(_BF16)
                for b in range(NB):
                    out = out + jnp.dot(
                        xm[b * H:(b + 1) * H],
                        w_ref[pl.ds(b * LW + n * PIECE, PIECE), :],
                        preferred_element_type=_F32)
            return out

        c_x.wait()
        x = x_v[0].astype(_F32)
        mu = jnp.mean(x, axis=-1, keepdims=True)
        xc = x - mu
        var = jnp.mean(xc * xc, axis=-1, keepdims=True)
        xn = xc * lax.rsqrt(var + 1e-5)
        xn_v[...] = jnp.broadcast_to(xn, (H, M)).astype(_BF16)
        xn_b = xn_v[...]

        c_w1.wait()
        c_wuk.start()
        h1 = lax.dot_general(xn_b[0:16], w1_v[...], _NT,
                             preferred_element_type=_F32)
        h1 = _silu(h1).astype(_BF16)
        c_w2.wait()
        g = _silu(jnp.dot(h1, w2_v[...], preferred_element_type=_F32))[0:8]

        c_wq.wait()
        c_kv[0].start()
        q = diag_contract(xn_b, wq_v).astype(_BF16)

        c_wuk.wait()
        c_kv[1].start()
        mask = head_mask(H)
        z = jnp.zeros((NB * H, 128), _F32)
        for n in range(LW // PIECE):
            ys = []
            for b in range(NB):
                t = lax.dot_general(
                    q, wuk_v[pl.ds(b * LW + n * PIECE, PIECE), :], _NT,
                    preferred_element_type=_F32)
                ys.append(jnp.where(mask, t * (D ** -0.5), 0.0).astype(_BF16))
            y = jnp.concatenate(ys, axis=0)
            z = z + lax.dot_general(y, e_v[:, n * PIECE:(n + 1) * PIECE], _NT,
                                    preferred_element_type=_F32)
        qa = jnp.concatenate(
            [z[b * H:(b + 1) * H] for b in range(NB)], axis=1).astype(_BF16)

        def tile(i, carry):
            m, l, acc = carry
            c = ckv_v[pl.ds(pl.multiple_of(i * T, T), T), :]
            s = lax.dot_general(qa, c, _NT, preferred_element_type=_F32)
            m_new = jnp.maximum(m, jnp.max(s, axis=-1, keepdims=True))
            alpha = jnp.exp(m - m_new)
            p = jnp.exp(s - m_new)
            l = l * alpha + jnp.sum(p, axis=-1, keepdims=True)
            acc = acc * alpha + jnp.dot(p.astype(_BF16), c,
                                        preferred_element_type=_F32)
            return m_new, l, acc

        carry = (jnp.full((H, 1), -jnp.inf, _F32), jnp.zeros((H, 1), _F32),
                 jnp.zeros((H, DC), _F32))
        later = c_kv[2:] + [c_wuv, c_wo[0]]
        off = 0
        for k, n in enumerate(KV_CHUNKS):
            c_kv[k].wait()
            later[k].start()
            carry = lax.fori_loop(off // T, (off + n) // T, tile, carry)
            off += n
        _, l, acc = carry
        ctx_c = (acc * (1.0 / l)).astype(_BF16)

        c_wuv.wait()
        c_wo[1].start()
        c_wo[2].start(priority=1)
        ctx = diag_contract(ctx_c, wuv_v)

        for h in range(H):
            lhs_v[:, h * D:(h + 1) * D] = jnp.broadcast_to(
                ctx[h:h + 1], (16, D)).astype(_BF16)
        s_out = jnp.zeros((16, M), _F32)
        for k, (a, b) in enumerate(zip(WO_SPLIT[:-1], WO_SPLIT[1:])):
            c_wo[k].wait()
            s_out = s_out + jnp.dot(lhs_v[:, a:b], wo_v[a:b, :],
                                    preferred_element_type=_F32)
        o_ref[0] = (x + s_out[0:1] * g[0:1]).astype(o_ref.dtype)

    n_sems = 6 + len(KV_CHUNKS) + len(WO_SPLIT) - 1
    any_spec = pl.BlockSpec(memory_space=pl.ANY)
    return pl.pallas_call(
        kernel,
        out_shape=jax.ShapeDtypeStruct(A_x.shape, A_x.dtype),
        in_specs=[any_spec] * 8,
        out_specs=pl.BlockSpec(memory_space=pltpu.VMEM),
        scratch_shapes=[
            pltpu.VMEM(A_x.shape, _BF16),
            pltpu.VMEM((S, DC), _BF16),
            pltpu.VMEM((M * H, D), _BF16),
            pltpu.VMEM((DC * H, D), _BF16),
            pltpu.VMEM((DC * H, D), _BF16),
            pltpu.VMEM((H * D, M), _BF16),
            pltpu.VMEM((F, M), _BF16),
            pltpu.VMEM((F, M), _BF16),
            pltpu.VMEM((128, LW), _BF16),
            pltpu.VMEM((H, M), _BF16),
            pltpu.VMEM((16, H * D), _BF16),
            pltpu.SemaphoreType.DMA((n_sems,)),
        ],
        compiler_params=pltpu.CompilerParams(vmem_limit_bytes=100 * 1024 * 1024),
    )(A_x, ckv2, wq2, wuk2, wuv2, wo2, w1t, B_w2)
```

```python
import jax
import jax.numpy as jnp
from jax import lax
import jax.experimental.pallas as pl
import jax.experimental.pallas.tpu as pltpu

_NT = (((1,), (1,)), ((), ()))
_F32 = jnp.float32
_BF16 = jnp.bfloat16


def _silu(v):
    return v * (1.0 / (1.0 + jnp.exp(-v)))


@jax.jit
def pallas_recurrent_scan__compressed_kv_cla__dense_activation_silu__decode_kernel(
    A_x: jax.Array,
    A_c_kv: jax.Array,
    A_w_q: jax.Array,
    A_w_uk: jax.Array,
    A_w_uv: jax.Array,
    A_w_o: jax.Array,
    B_x: jax.Array,
    B_w1: jax.Array,
    B_w2: jax.Array,
):
    del B_x
    B, Sq, M = A_x.shape
    _, S, DC = A_c_kv.shape
    _, H, D = A_w_q.shape
    F = B_w1.shape[1]
    assert B == 1 and Sq == 1 and D == 128 and H == 32 and M == 512 and DC == 512

    T = 2048
    NT = S // T
    NB = 4
    LW = 128 * H
    PIECE = 512
    NP = LW // PIECE
    WO_SPLIT = (0, 20 * D, 28 * D, 31 * D, 32 * D)
    N_WO = len(WO_SPLIT) - 1

    ckv2 = A_c_kv.reshape(S, DC)
    wq2 = A_w_q.reshape(M * H, D)
    wuk2 = A_w_uk.reshape(DC * H, D)
    wuv2 = A_w_uv.reshape(DC * H, D)
    wo2 = A_w_o.reshape(H * D, M)
    w1t = B_w1.T

    def kernel(x_hbm, ckv_hbm, wq_hbm, wuk_hbm, wuv_hbm, wo_hbm, w1_hbm, w2_hbm,
               o_ref,
               x_v, ckv_v, wq_v, wuk_v, wuv_v, wo_v, w1_v, w2_v,
               e_v, a_v, xm_v, lhs_v, s_v, sems, kv_sems, wo_sems):
        c_x = pltpu.make_async_copy(x_hbm, x_v, sems.at[0])
        c_wq = pltpu.make_async_copy(wq_hbm, wq_v, sems.at[1])
        c_wuk = pltpu.make_async_copy(wuk_hbm, wuk_v, sems.at[2])
        c_w1 = pltpu.make_async_copy(w1_hbm, w1_v, sems.at[3])
        c_w2 = pltpu.make_async_copy(w2_hbm, w2_v, sems.at[4])
        c_wuv = pltpu.make_async_copy(wuv_hbm, wuv_v, sems.at[5])

        def c_kv(i):
            rows = pl.ds(pl.multiple_of(i * T, T), T)
            return pltpu.make_async_copy(
                ckv_hbm.at[rows], ckv_v.at[rows], kv_sems.at[i])

        c_wo = [
            pltpu.make_async_copy(wo_hbm.at[pl.ds(a, b - a)],
                                  wo_v.at[pl.ds(a, b - a)], wo_sems.at[k])
            for k, (a, b) in enumerate(zip(WO_SPLIT[:-1], WO_SPLIT[1:]))
        ]

        c_x.start()
        c_wq.start()
        c_wuk.start()
        c_w1.start()
        c_w2.start()

        def start_kv(i, carry):
            c_kv(i).start()
            return carry

        lax.fori_loop(0, NT, start_kv, 0)
        c_wuv.start()

        def build_e(n, carry):
            row = lax.broadcasted_iota(jnp.int32, (128, PIECE), 0)
            col = lax.broadcasted_iota(jnp.int32, (128, PIECE), 1) + n * PIECE
            e_v[n] = jnp.where(row == (col >> 5), 1.0, 0.0).astype(_BF16)
            return carry

        lax.fori_loop(0, NP, build_e, 0)
        for c in c_wo:
            c.start()

        def head_mask(rows):
            r = lax.broadcasted_iota(jnp.int32, (rows, PIECE), 0)
            c = lax.broadcasted_iota(jnp.int32, (rows, PIECE), 1)
            return (r & (H - 1)) == (c & (H - 1))

        def expand(a):
            for b in range(NB):
                a_v[b * H:(b + 1) * H, :] = a[:, b * 128:(b + 1) * 128]

            def body(n, carry):
                r = jnp.dot(a_v[...], e_v[n], preferred_element_type=_F32)
                xm_v[n] = jnp.where(head_mask(NB * H), r, 0.0).astype(_BF16)
                return carry

            lax.fori_loop(0, NP, body, 0)

        def contract(w_ref):
            def body(n, out):
                for b in range(NB):
                    rows = pl.ds(pl.multiple_of(b * LW + n * PIECE, PIECE), PIECE)
                    out = out + jnp.dot(xm_v[n, b * H:(b + 1) * H, :],
                                        w_ref[rows, :],
                                        preferred_element_type=_F32)
                return out

            return lax.fori_loop(0, NP, body, jnp.zeros((H, D), _F32))

        c_x.wait()
        x = x_v[0].astype(_F32)
        mu = jnp.mean(x, axis=-1, keepdims=True)
        xc = x - mu
        var = jnp.mean(xc * xc, axis=-1, keepdims=True)
        xn = xc * lax.rsqrt(var + 1e-5)
        lhs_v[:, 0:M] = jnp.broadcast_to(xn, (16, M)).astype(_BF16)
        xn16 = lhs_v[:, 0:M]
        expand(jnp.concatenate([xn16, xn16], axis=0))

        c_wq.wait()
        q = contract(wq_v).astype(_BF16)

        c_wuk.wait()

        def absorb(n, z):
            ys = []
            for b in range(NB):
                rows = pl.ds(pl.multiple_of(b * LW + n * PIECE, PIECE), PIECE)
                t = lax.dot_general(q, wuk_v[rows, :], _NT,
                                    preferred_element_type=_F32)
                ys.append(jnp.where(head_mask(H), t * (D ** -0.5), 0.0)
                          .astype(_BF16))
            y = jnp.concatenate(ys, axis=0)
            return z + lax.dot_general(y, e_v[n], _NT,
                                       preferred_element_type=_F32)

        z = lax.fori_loop(0, NP, absorb, jnp.zeros((NB * H, 128), _F32))
        qa = jnp.concatenate(
            [z[b * H:(b + 1) * H] for b in range(NB)], axis=1).astype(_BF16)

        c_w1.wait()
        h1 = lax.dot_general(xn16, w1_v[...], _NT, preferred_element_type=_F32)
        h1 = _silu(h1).astype(_BF16)
        c_w2.wait()
        g = _silu(jnp.dot(h1, w2_v[...], preferred_element_type=_F32))[0:8]

        def tile(i, carry):
            m, l, acc = carry
            c_kv(i).wait()
            c = ckv_v[pl.ds(pl.multiple_of(i * T, T), T), :]
            s = lax.dot_general(qa, c, _NT, preferred_element_type=_F32)
            m_new = jnp.maximum(m, jnp.max(s, axis=-1, keepdims=True))
            alpha = jnp.exp(m - m_new)
            p = jnp.exp(s - m_new)
            l = l * alpha + jnp.sum(p, axis=-1, keepdims=True)
            acc = acc * alpha + jnp.dot(p.astype(_BF16), c,
                                        preferred_element_type=_F32)
            return m_new, l, acc

        carry = (jnp.full((H, 1), -jnp.inf, _F32), jnp.zeros((H, 1), _F32),
                 jnp.zeros((H, DC), _F32))
        _, l, acc = lax.fori_loop(0, NT, tile, carry)
        expand((acc * (1.0 / l)).astype(_BF16))

        c_wuv.wait()
        ctx = contract(wuv_v)

        for h in range(H):
            lhs_v[:, h * D:(h + 1) * D] = jnp.broadcast_to(
                ctx[h:h + 1], (16, D)).astype(_BF16)
        for k, (a, b) in enumerate(zip(WO_SPLIT[:-1], WO_SPLIT[1:])):
            c_wo[k].wait()
            part = jnp.dot(lhs_v[:, a:b], wo_v[a:b, :],
                           preferred_element_type=_F32)[0:8]
            if k == 0:
                s_v[...] = part
            elif k < N_WO - 1:
                s_v[...] += part
            else:
                s_out = s_v[...] + part
        o_ref[0] = (x + s_out[0:1] * g[0:1]).astype(o_ref.dtype)

    any_spec = pl.BlockSpec(memory_space=pl.ANY)
    return pl.pallas_call(
        kernel,
        out_shape=jax.ShapeDtypeStruct(A_x.shape, A_x.dtype),
        in_specs=[any_spec] * 8,
        out_specs=pl.BlockSpec(memory_space=pltpu.VMEM),
        scratch_shapes=[
            pltpu.VMEM(A_x.shape, _BF16),
            pltpu.VMEM((S, DC), _BF16),
            pltpu.VMEM((M * H, D), _BF16),
            pltpu.VMEM((DC * H, D), _BF16),
            pltpu.VMEM((DC * H, D), _BF16),
            pltpu.VMEM((H * D, M), _BF16),
            pltpu.VMEM((F, M), _BF16),
            pltpu.VMEM((F, M), _BF16),
            pltpu.VMEM((NP, 128, PIECE), _BF16),
            pltpu.VMEM((NB * H, 128), _BF16),
            pltpu.VMEM((NP, NB * H, PIECE), _BF16),
            pltpu.VMEM((16, H * D), _BF16),
            pltpu.VMEM((8, M), _F32),
            pltpu.SemaphoreType.DMA((6,)),
            pltpu.SemaphoreType.DMA((NT,)),
            pltpu.SemaphoreType.DMA((N_WO,)),
        ],
        compiler_params=pltpu.CompilerParams(
            vmem_limit_bytes=100 * 1024 * 1024,
            disable_semaphore_checks=True),
    )(A_x, ckv2, wq2, wuk2, wuv2, wo2, w1t, B_w2)
```

```python
import jax
import jax.numpy as jnp
from jax import lax
import jax.experimental.pallas as pl
import jax.experimental.pallas.tpu as pltpu

_NT = (((1,), (1,)), ((), ()))
_F32 = jnp.float32
_BF16 = jnp.bfloat16


def _silu(v):
    return v * (1.0 / (1.0 + jnp.exp(-v)))


def _compiler_params():
    limit = 100 * 1024 * 1024
    try:
        return pltpu.CompilerParams(vmem_limit_bytes=limit,
                                    disable_semaphore_checks=True)
    except TypeError:
        return pltpu.CompilerParams(vmem_limit_bytes=limit)


@jax.jit
def pallas_recurrent_scan__compressed_kv_cla__dense_activation_silu__decode_kernel(
    A_x: jax.Array,
    A_c_kv: jax.Array,
    A_w_q: jax.Array,
    A_w_uk: jax.Array,
    A_w_uv: jax.Array,
    A_w_o: jax.Array,
    B_x: jax.Array,
    B_w1: jax.Array,
    B_w2: jax.Array,
):
    del B_x
    B, Sq, M = A_x.shape
    _, S, DC = A_c_kv.shape
    _, H, D = A_w_q.shape
    F = B_w1.shape[1]
    assert B == 1 and Sq == 1 and D == 128 and H == 32 and M == 512 and DC == 512

    T = 2048
    NT = S // T
    assert NT * T == S
    NB = 4
    LW = 128 * H
    PIECE = 512
    NP = LW // PIECE

    CH = 64
    PRE = (2, 2, 1, 1)
    POST = 2
    AHEAD = 2
    RING = 2 * AHEAD
    NCH = sum(PRE) + NT + POST
    RS = NCH * CH
    WO_SPLIT = (RS, 20 * D, 28 * D, 30 * D, 31 * D,
                31 * D + 80, 31 * D + 112, 32 * D)
    N_WO = len(WO_SPLIT) - 1
    N_MXU = 4
    assert RS % D == 0 and RS < WO_SPLIT[1] and POST >= AHEAD and N_WO < NT

    ckv2 = A_c_kv.reshape(S, DC)
    wq2 = A_w_q.reshape(M * H, D)
    wuk2 = A_w_uk.reshape(DC * H, D)
    wuv2 = A_w_uv.reshape(DC * H, D)
    wo2 = A_w_o.reshape(H * D, M)
    w1t = B_w1.T

    def kernel(x_hbm, ckv_hbm, wq_hbm, wuk_hbm, wuv_hbm, wo_hbm, w1_hbm, w2_hbm,
               o_ref,
               x_v, ckv_v, wq_v, wuk_v, wuv_v, wo_v, w1_v, w2_v,
               e_v, a_v, xm_v, lhs_v, s_v, cb_v, mult_v, stage,
               sems, kv_sems, wo_sems, h2s_sems, s2v_sems):
        c_x = pltpu.make_async_copy(x_hbm, x_v, sems.at[0])
        c_wq = pltpu.make_async_copy(wq_hbm, wq_v, sems.at[1])
        c_wuk = pltpu.make_async_copy(wuk_hbm, wuk_v, sems.at[2])
        c_w1 = pltpu.make_async_copy(w1_hbm, w1_v, sems.at[3])
        c_w2 = pltpu.make_async_copy(w2_hbm, w2_v, sems.at[4])
        c_wuv = pltpu.make_async_copy(wuv_hbm, wuv_v, sems.at[5])

        def c_kv(i):
            rows = pl.ds(pl.multiple_of(i * T, T), T)
            return pltpu.make_async_copy(
                ckv_hbm.at[rows], ckv_v.at[rows], kv_sems.at[i])

        c_wo = [
            pltpu.make_async_copy(wo_hbm.at[pl.ds(a, b - a)],
                                  wo_v.at[pl.ds(a, b - a)], wo_sems.at[k])
            for k, (a, b) in enumerate(zip(WO_SPLIT[:-1], WO_SPLIT[1:]))
        ]

        def chunk_rows(j):
            if isinstance(j, int):
                return pl.ds(j * CH, CH)
            return pl.ds(pl.multiple_of(j * CH, CH), CH)

        def h2s(j):
            slot = j % RING
            return pltpu.make_async_copy(
                wo_hbm.at[chunk_rows(j)], stage.at[slot], h2s_sems.at[slot])

        def s2v(j):
            slot = j % RING
            return pltpu.make_async_copy(
                stage.at[slot], wo_v.at[chunk_rows(j)], s2v_sems.at[slot])

        def tick(j):
            static = isinstance(j, int)
            h2s(j).wait()
            s2v(j).start()
            if not static or j + AHEAD < NCH:
                if not static or j >= AHEAD:
                    s2v(j - AHEAD).wait()
                h2s(j + AHEAD).start()

        def ticks(j0, n):
            for j in range(j0, j0 + n):
                tick(j)
            return j0 + n

        c_x.start()
        c_wq.start()
        for j in range(AHEAD):
            h2s(j).start()
        c_wuk.start()
        c_w1.start()
        c_w2.start()

        def start_kv(i, carry):
            c_kv(i).start()
            return carry

        lax.fori_loop(0, NT, start_kv, 0)

        def build_e(n, carry):
            row = lax.broadcasted_iota(jnp.int32, (128, PIECE), 0)
            col = lax.broadcasted_iota(jnp.int32, (128, PIECE), 1) + n * PIECE
            e_v[n] = jnp.where(row == (col >> 5), 1.0, 0.0).astype(_BF16)
            return carry

        lax.fori_loop(0, NP, build_e, 0)

        def head_mask(rows):
            r = lax.broadcasted_iota(jnp.int32, (rows, PIECE), 0)
            c = lax.broadcasted_iota(jnp.int32, (rows, PIECE), 1)
            return (r & (H - 1)) == (c & (H - 1))

        def expand(a):
            for b in range(NB):
                a_v[b * H:(b + 1) * H, :] = a[:, b * 128:(b + 1) * 128]

            def body(n, carry):
                r = jnp.dot(a_v[...], e_v[n], preferred_element_type=_F32)
                xm_v[n] = jnp.where(head_mask(NB * H), r, 0.0).astype(_BF16)
                return carry

            lax.fori_loop(0, NP, body, 0)

        def contract(w_ref):
            def body(n, out):
                for b in range(NB):
                    rows = pl.ds(pl.multiple_of(b * LW + n * PIECE, PIECE), PIECE)
                    out = out + jnp.dot(xm_v[n, b * H:(b + 1) * H, :],
                                        w_ref[rows, :],
                                        preferred_element_type=_F32)
                return out

            return lax.fori_loop(0, NP, body, jnp.zeros((H, D), _F32))

        c_x.wait()
        x = x_v[0].astype(_F32)
        mu = jnp.mean(x, axis=-1, keepdims=True)
        xc = x - mu
        var = jnp.mean(xc * xc, axis=-1, keepdims=True)
        xn = xc * lax.rsqrt(var + 1e-5)
        lhs_v[:, 0:M] = jnp.broadcast_to(xn, (16, M)).astype(_BF16)
        xn16 = lhs_v[:, 0:M]
        expand(jnp.concatenate([xn16, xn16], axis=0))
        j = ticks(0, PRE[0])

        c_wq.wait()
        q = contract(wq_v).astype(_BF16)
        j = ticks(j, PRE[1])

        c_wuk.wait()

        def absorb(n, z):
            ys = []
            for b in range(NB):
                rows = pl.ds(pl.multiple_of(b * LW + n * PIECE, PIECE), PIECE)
                t = lax.dot_general(q, wuk_v[rows, :], _NT,
                                    preferred_element_type=_F32)
                ys.append(jnp.where(head_mask(H), t * (D ** -0.5), 0.0)
                          .astype(_BF16))
            y = jnp.concatenate(ys, axis=0)
            return z + lax.dot_general(y, e_v[n], _NT,
                                       preferred_element_type=_F32)

        z = lax.fori_loop(0, NP, absorb, jnp.zeros((NB * H, 128), _F32))
        qa = jnp.concatenate(
            [z[b * H:(b + 1) * H] for b in range(NB)], axis=1).astype(_BF16)
        j = ticks(j, PRE[2])

        c_w1.wait()
        h1 = lax.dot_general(xn16, w1_v[...], _NT, preferred_element_type=_F32)
        h1 = _silu(h1).astype(_BF16)
        c_w2.wait()
        g = _silu(jnp.dot(h1, w2_v[...], preferred_element_type=_F32))[0:8]
        j_loop = ticks(j, PRE[3])

        def tile(i, carry):
            m, l, acc = carry
            c_kv(i).wait()
            for k, c in enumerate([c_wuv] + c_wo):
                pl.when(i == k)(c.start)
            tick(i + j_loop)
            c = ckv_v[pl.ds(pl.multiple_of(i * T, T), T), :]
            s = lax.dot_general(qa, c, _NT, preferred_element_type=_F32)
            m_new = jnp.maximum(m, jnp.max(s, axis=-1, keepdims=True))
            alpha = jnp.exp(m - m_new)
            p = jnp.exp(s - m_new)
            l = l * alpha + jnp.sum(p, axis=-1, keepdims=True)
            acc = acc * alpha + jnp.dot(p.astype(_BF16), c,
                                        preferred_element_type=_F32)
            return m_new, l, acc

        init = (jnp.full((H, 1), -jnp.inf, _F32), jnp.zeros((H, 1), _F32),
                jnp.zeros((H, DC), _F32))
        _, l, acc = lax.fori_loop(0, NT, tile, init)
        expand((acc * (1.0 / l)).astype(_BF16))
        ticks(j_loop + NT, POST)

        c_wuv.wait()
        ctx = contract(wuv_v).astype(_BF16).astype(_F32)

        for h in range(H - 1):
            lhs_v[:, h * D:(h + 1) * D] = jnp.broadcast_to(
                ctx[h:h + 1], (16, D)).astype(_BF16)
        cb_v[...] = jnp.broadcast_to(ctx[H - 1:H], (D, D))
        cb = cb_v[...].T
        for b in range(NB):
            mult_v[:, b * 128:(b + 1) * 128] = cb * g[0:1, b * 128:(b + 1) * 128]

        for jj in range(NCH - RING, NCH):
            s2v(jj).wait()
        s_v[...] = jnp.dot(lhs_v[:, 0:RS], wo_v[0:RS, :],
                           preferred_element_type=_F32)[0:8]
        for k, (a, b) in enumerate(zip(WO_SPLIT[:-1], WO_SPLIT[1:])):
            c_wo[k].wait()
            if k < N_MXU:
                part = jnp.dot(lhs_v[:, a:b], wo_v[a:b, :],
                               preferred_element_type=_F32)[0:8]
                if k < N_MXU - 1:
                    s_v[...] += part
                else:
                    base = jnp.broadcast_to(x, (8, M)) + (s_v[...] + part) * g
                    row0 = lax.broadcasted_iota(jnp.int32, (8, M), 0) == 0
                    s_v[...] = jnp.where(row0, base, 0.0)
            else:
                r0 = a - (H - 1) * D
                prod = wo_v[a:b, :].astype(_F32) * mult_v[r0:r0 + b - a, :]
                parts = [s_v[...]] + [prod[r:r + 8] for r in range(0, b - a, 8)]
                while len(parts) > 1:
                    parts = [parts[i] + parts[i + 1] if i + 1 < len(parts)
                             else parts[i] for i in range(0, len(parts), 2)]
                if k < N_WO - 1:
                    s_v[...] = parts[0]
                else:
                    o_ref[0] = jnp.sum(parts[0], axis=0,
                                       keepdims=True).astype(o_ref.dtype)

    any_spec = pl.BlockSpec(memory_space=pl.ANY)
    return pl.pallas_call(
        kernel,
        out_shape=jax.ShapeDtypeStruct(A_x.shape, A_x.dtype),
        in_specs=[any_spec] * 8,
        out_specs=pl.BlockSpec(memory_space=pltpu.VMEM),
        scratch_shapes=[
            pltpu.VMEM(A_x.shape, _BF16),
            pltpu.VMEM((S, DC), _BF16),
            pltpu.VMEM((M * H, D), _BF16),
            pltpu.VMEM((DC * H, D), _BF16),
            pltpu.VMEM((DC * H, D), _BF16),
            pltpu.VMEM((H * D, M), _BF16),
            pltpu.VMEM((F, M), _BF16),
            pltpu.VMEM((F, M), _BF16),
            pltpu.VMEM((NP, 128, PIECE), _BF16),
            pltpu.VMEM((NB * H, 128), _BF16),
            pltpu.VMEM((NP, NB * H, PIECE), _BF16),
            pltpu.VMEM((16, H * D), _BF16),
            pltpu.VMEM((8, M), _F32),
            pltpu.VMEM((D, D), _F32),
            pltpu.VMEM((D, M), _F32),
            pltpu.SMEM((RING, CH, M), _BF16),
            pltpu.SemaphoreType.DMA((6,)),
            pltpu.SemaphoreType.DMA((NT,)),
            pltpu.SemaphoreType.DMA((N_WO,)),
            pltpu.SemaphoreType.DMA((RING,)),
            pltpu.SemaphoreType.DMA((RING,)),
        ],
        compiler_params=_compiler_params(),
    )(A_x, ckv2, wq2, wuk2, wuv2, wo2, w1t, B_w2)
```

```python
import jax
import jax.numpy as jnp
from jax import lax
import jax.experimental.pallas as pl
import jax.experimental.pallas.tpu as pltpu

_NT = (((1,), (1,)), ((), ()))
_F32 = jnp.float32
_BF16 = jnp.bfloat16


def _silu(v):
    return v * (1.0 / (1.0 + jnp.exp(-v)))


def _compiler_params():
    limit = 100 * 1024 * 1024
    try:
        return pltpu.CompilerParams(vmem_limit_bytes=limit,
                                    disable_semaphore_checks=True)
    except TypeError:
        return pltpu.CompilerParams(vmem_limit_bytes=limit)


@jax.jit
def pallas_recurrent_scan__compressed_kv_cla__dense_activation_silu__decode_kernel(
    A_x: jax.Array,
    A_c_kv: jax.Array,
    A_w_q: jax.Array,
    A_w_uk: jax.Array,
    A_w_uv: jax.Array,
    A_w_o: jax.Array,
    B_x: jax.Array,
    B_w1: jax.Array,
    B_w2: jax.Array,
):
    del B_x
    B, Sq, M = A_x.shape
    _, S, DC = A_c_kv.shape
    _, H, D = A_w_q.shape
    F = B_w1.shape[1]
    assert (B, Sq, M, S, DC, H, D, F) == (1, 1, 512, 32768, 512, 32, 128, 1376)

    NB = 4
    G = 16
    NP = 128 // G

    KR, KA, KB = 48, 4, 17
    T = 1920
    NT = S // T
    SM = NT * T
    REM = S - SM
    NR = SM // (KA * KB * KR)
    DPT = T // (KA * KR)
    assert NR * KA * KB * KR == SM and DPT * KA * KR == T
    KW = 2
    WA, WB, WR = 5, 17, 192
    WM = WA * WB * WR
    WN = M * H
    GRP = (0, 4, 8, 12, 17)
    GW = 4

    CH, N1, AHEAD = 32, 6, 6
    RING = 2 * AHEAD
    NCH = N1 + F // CH
    R1 = N1 * CH
    TPI = 2

    WO_SPLIT = (0, 16 * D, 26 * D, 30 * D, 31 * D,
                31 * D + 80, 31 * D + 112, 32 * D)
    N_WO = len(WO_SPLIT) - 1
    N_MXU = 4
    WPI = -(-N_WO // KW)

    ckv2 = A_c_kv.reshape(S, DC)
    wq2 = A_w_q.reshape(WN, D)
    wuk2 = A_w_uk.reshape(WN, D)
    wuv2 = A_w_uv.reshape(WN, D)
    wo2 = A_w_o.reshape(H * D, M)
    w1t = B_w1.T

    def kernel(x_hbm, ckv_hbm, wq_hbm, wuk_hbm, wuv_hbm, wo_hbm, w1_hbm, w2_hbm,
               o_ref,
               x_v, ckv_v, rem_v, wq_v, wuk_v, wuv_v, wrest_v, wo_v, w1_v, w2_v,
               lhs_v, s_v, h_v, cb_v, af_v, mult_v, stage,
               sems, g_sems, kv_sems, wo_sems, h2s_sems, s2v_sems):
        c_x = pltpu.make_async_copy(x_hbm, x_v, sems.at[0])
        c_w1 = pltpu.make_async_copy(w1_hbm.at[pl.ds(R1, F - R1)],
                                     w1_v.at[pl.ds(R1, F - R1)], sems.at[1])
        c_rem = pltpu.make_async_copy(ckv_hbm.at[pl.ds(SM, REM)], rem_v,
                                      sems.at[2])
        ws = [(wq_hbm, wq_v), (wuk_hbm, wuk_v), (wuv_hbm, wuv_v)]
        NG = 4 * len(ws)

        def w_rest(g):
            return pltpu.make_async_copy(
                ws[g // 4][0].at[pl.ds(WM, WN - WM)], wrest_v.at[g // 4],
                g_sems.at[g])

        def start_group(g):
            src, dst = ws[g // 4]

            def body(b, carry):
                view = src.at[pl.ds(0, WM)].reshape(WA, WB, WR, D)
                pltpu.make_async_copy(view.at[:, b], dst.at[b],
                                      g_sems.at[g]).start()
                return carry

            lax.fori_loop(GRP[g % 4], GRP[g % 4 + 1], body, 0)
            if g % 4 == 0:
                w_rest(g).start()

        def wait_group(g):
            lo, hi = GRP[g % 4], GRP[g % 4 + 1]
            region = ws[g // 4][1].at[pl.ds(lo, hi - lo)]
            pltpu.make_async_copy(region, region, g_sems.at[g]).wait()
            if g % 4 == 0:
                w_rest(g).wait()

        def start_tile(i):
            def body(d, carry):
                view = ckv_hbm.at[pl.ds(0, SM)].reshape(NR, KA, KB, KR, DC)
                pltpu.make_async_copy(
                    view.at[d // KB, :, d % KB], ckv_v.at[pl.ds(d * KA, KA)],
                    kv_sems.at[i]).start()
                return carry

            lax.fori_loop(i * DPT, (i + 1) * DPT, body, 0)

        def tile_ref(i):
            return ckv_v.at[pl.ds(i * (T // KR), T // KR)]

        def wait_tile(i):
            pltpu.make_async_copy(tile_ref(i), tile_ref(i),
                                  kv_sems.at[i]).wait()

        c_wo = [
            pltpu.make_async_copy(wo_hbm.at[pl.ds(a, b - a)],
                                  wo_v.at[pl.ds(a, b - a)], wo_sems.at[k])
            for k, (a, b) in enumerate(zip(WO_SPLIT[:-1], WO_SPLIT[1:]))
        ]

        def step(g):
            wait_group(g)
            if g + GW < NG:
                start_group(g + GW)
            elif g == NG - 3:
                c_rem.start()
                start_tile(0)
            elif g == NG - 1:
                start_tile(1)

        def chunk(j):
            if isinstance(j, int):
                if j < N1:
                    return w1_hbm, w1_v, pl.ds(j * CH, CH)
                return w2_hbm, w2_v, pl.ds((j - N1) * CH, CH)
            return w2_hbm, w2_v, pl.ds(pl.multiple_of((j - N1) * CH, CH), CH)

        def h2s(j):
            src, _, rows = chunk(j)
            slot = j % RING
            return pltpu.make_async_copy(
                src.at[rows], stage.at[slot], h2s_sems.at[slot])

        def s2v(j):
            _, dst, rows = chunk(j)
            slot = j % RING
            return pltpu.make_async_copy(
                stage.at[slot], dst.at[rows], s2v_sems.at[slot])

        def tick(j):
            h2s(j).wait()
            s2v(j).start()
            if isinstance(j, int):
                if j + AHEAD < NCH:
                    if j >= AHEAD:
                        s2v(j - AHEAD).wait()
                    h2s(j + AHEAD).start()
            else:
                @pl.when(j + AHEAD < NCH)
                def _():
                    s2v(j - AHEAD).wait()
                    h2s(j + AHEAD).start()

        def slab(wi, c):
            spp = WR // H
            k = c // spp
            if k >= WA * WB:
                r = (c - WA * WB * spp) * H
                return wrest_v[wi, r:r + H, :]
            r = (c % spp) * H
            return ws[wi][1][k % WB, k // WB, r:r + H, :]

        def w_tiles(wi, n):
            return jnp.concatenate(
                [slab(wi, 128 * b + n * G + jj) for jj in range(G)
                 for b in range(NB)], axis=0)

        def head_mask(cols):
            r = lax.broadcasted_iota(jnp.int32, (H, cols), 0)
            c = lax.broadcasted_iota(jnp.int32, (H, cols), 1)
            return r == (c & (H - 1))

        def contract(a, wi):
            for b in range(NB):
                cb_v[b * H:(b + 1) * H, :] = a[:, b * 128:(b + 1) * 128]
            af_v[...] = cb_v[...].T
            mask = head_mask(128)
            out = jnp.zeros((H, D), _F32)
            for n in range(NP):
                lhs = jnp.concatenate(
                    [jnp.where(mask, af_v[pl.ds(n * G + jj, 1), :], 0.0)
                     .astype(_BF16) for jj in range(G)], axis=1)
                out = out + jnp.dot(lhs, w_tiles(wi, n),
                                    preferred_element_type=_F32)
            return out

        c_w1.start()
        for j in range(AHEAD):
            h2s(j).start()
        c_x.start()
        for g in range(GW):
            start_group(g)
        c_w1.wait()
        tick(0)
        for g in range(8):
            step(g)
            tick(g + 1)

        c_x.wait()
        x = x_v[0].astype(_F32)
        mu = jnp.mean(x, axis=-1, keepdims=True)
        xc = x - mu
        var = jnp.mean(xc * xc, axis=-1, keepdims=True)
        xn = xc * lax.rsqrt(var + 1e-5)
        lhs_v[:, 0:M] = jnp.broadcast_to(xn, (16, M)).astype(_BF16)
        xn16 = lhs_v[:, 0:M]
        q = contract(jnp.concatenate([xn16, xn16], axis=0).astype(_F32),
                     0).astype(_BF16)
        step(8)
        tick(9)

        for n in range(NP):
            t = lax.dot_general(q, w_tiles(1, n), _NT,
                                preferred_element_type=_F32)
            r = jnp.sum(jnp.where(head_mask(G * 128), t, 0.0), axis=0,
                        keepdims=True)
            for jj in range(G):
                af_v[pl.ds(n * G + jj, 1), :] = r[:, jj * 128:(jj + 1) * 128]
            if n == NP // 2 - 1:
                step(9)
                tick(10)
        z = af_v[...].T * (D ** -0.5)
        qa = jnp.concatenate(
            [z[b * H:(b + 1) * H] for b in range(NB)], axis=1).astype(_BF16)
        step(10)
        tick(11)
        step(11)
        tick(12)
        j_loop = 13
        assert j_loop - AHEAD >= N1 and j_loop + TPI * NT <= NCH

        h1 = lax.dot_general(xn16, w1_v[...], _NT, preferred_element_type=_F32)
        h_v[...] = _silu(h1).astype(_BF16)

        c_rem.wait()
        c0 = rem_v[...]
        s0 = lax.dot_general(qa, c0, _NT, preferred_element_type=_F32)
        m0 = jnp.max(s0, axis=-1, keepdims=True)
        p0 = jnp.exp(s0 - m0)
        init = (m0, jnp.sum(p0, axis=-1, keepdims=True),
                jnp.dot(p0.astype(_BF16), c0, preferred_element_type=_F32))

        def tile(i, carry):
            m, l, acc = carry
            wait_tile(i)

            @pl.when(i + KW < NT)
            def _():
                start_tile(i + KW)

            for k, cp in enumerate(c_wo):
                pl.when(i == NT - KW + k // WPI)(cp.start)
            for t in range(TPI):
                tick(i * TPI + t + j_loop)
            c = tile_ref(i)[...].reshape(T, DC)
            s = lax.dot_general(qa, c, _NT, preferred_element_type=_F32)
            m_new = jnp.maximum(m, jnp.max(s, axis=-1, keepdims=True))
            alpha = jnp.exp(m - m_new)
            p = jnp.exp(s - m_new)
            l = l * alpha + jnp.sum(p, axis=-1, keepdims=True)
            acc = acc * alpha + jnp.dot(p.astype(_BF16), c,
                                        preferred_element_type=_F32)
            return m_new, l, acc

        _, l, acc = lax.fori_loop(0, NT, tile, init)
        for j in range(j_loop + TPI * NT, NCH):
            tick(j)

        ctx = contract((acc * (1.0 / l)).astype(_BF16).astype(_F32),
                       2).astype(_BF16).astype(_F32)
        for h in range(H - 1):
            lhs_v[:, h * D:(h + 1) * D] = jnp.broadcast_to(
                ctx[h:h + 1], (16, D)).astype(_BF16)
        cb_v[...] = jnp.broadcast_to(ctx[H - 1:H], (D, D))
        af_v[...] = cb_v[...].T

        for k, (a, b) in enumerate(zip(WO_SPLIT[:-1], WO_SPLIT[1:])):
            if k == 1:
                for j in range(NCH - RING, NCH):
                    s2v(j).wait()
                g = _silu(jnp.dot(h_v[...], w2_v[...],
                                  preferred_element_type=_F32)[0:8])
                for bb in range(NB):
                    mult_v[:, bb * 128:(bb + 1) * 128] = (
                        af_v[...] * g[0:1, bb * 128:(bb + 1) * 128])
            c_wo[k].wait()
            if k < N_MXU:
                part = jnp.dot(lhs_v[:, a:b], wo_v[a:b, :],
                               preferred_element_type=_F32)[0:8]
                if k == 0:
                    s_v[...] = part
                elif k < N_MXU - 1:
                    s_v[...] += part
                else:
                    base = jnp.broadcast_to(x, (8, M)) + (s_v[...] + part) * g
                    row0 = lax.broadcasted_iota(jnp.int32, (8, M), 0) == 0
                    s_v[...] = jnp.where(row0, base, 0.0)
            else:
                r0 = a - (H - 1) * D
                prod = wo_v[a:b, :].astype(_F32) * mult_v[r0:r0 + b - a, :]
                parts = [s_v[...]] + [prod[r:r + 8] for r in range(0, b - a, 8)]
                while len(parts) > 1:
                    parts = [parts[i] + parts[i + 1] if i + 1 < len(parts)
                             else parts[i] for i in range(0, len(parts), 2)]
                if k < N_WO - 1:
                    s_v[...] = parts[0]
                else:
                    o_ref[0] = jnp.sum(parts[0], axis=0,
                                       keepdims=True).astype(o_ref.dtype)

    any_spec = pl.BlockSpec(memory_space=pl.ANY)
    return pl.pallas_call(
        kernel,
        out_shape=jax.ShapeDtypeStruct(A_x.shape, A_x.dtype),
        in_specs=[any_spec] * 8,
        out_specs=pl.BlockSpec(memory_space=pltpu.VMEM),
        scratch_shapes=[
            pltpu.VMEM(A_x.shape, _BF16),
            pltpu.VMEM((SM // KR, KR, DC), _BF16),
            pltpu.VMEM((REM, DC), _BF16),
            pltpu.VMEM((WB, WA, WR, D), _BF16),
            pltpu.VMEM((WB, WA, WR, D), _BF16),
            pltpu.VMEM((WB, WA, WR, D), _BF16),
            pltpu.VMEM((3, WN - WM, D), _BF16),
            pltpu.VMEM((H * D, M), _BF16),
            pltpu.VMEM((F, M), _BF16),
            pltpu.VMEM((F, M), _BF16),
            pltpu.VMEM((16, H * D), _BF16),
            pltpu.VMEM((8, M), _F32),
            pltpu.VMEM((16, F), _BF16),
            pltpu.VMEM((D, D), _F32),
            pltpu.VMEM((D, D), _F32),
            pltpu.VMEM((D, M), _F32),
            pltpu.SMEM((RING, CH, M), _BF16),
            pltpu.SemaphoreType.DMA((3,)),
            pltpu.SemaphoreType.DMA((12,)),
            pltpu.SemaphoreType.DMA((NT,)),
            pltpu.SemaphoreType.DMA((N_WO,)),
            pltpu.SemaphoreType.DMA((RING,)),
            pltpu.SemaphoreType.DMA((RING,)),
        ],
        compiler_params=_compiler_params(),
    )(A_x, ckv2, wq2, wuk2, wuv2, wo2, w1t, B_w2)
```

```python
import jax
import jax.numpy as jnp
from jax import lax
import jax.experimental.pallas as pl
import jax.experimental.pallas.tpu as pltpu

_NT = (((1,), (1,)), ((), ()))
_F32 = jnp.float32
_BF16 = jnp.bfloat16


def _silu(v):
    return v * (1.0 / (1.0 + jnp.exp(-v)))


def _compiler_params():
    limit = 100 * 1024 * 1024
    try:
        return pltpu.CompilerParams(vmem_limit_bytes=limit,
                                    disable_semaphore_checks=True)
    except TypeError:
        return pltpu.CompilerParams(vmem_limit_bytes=limit)


@jax.jit
def pallas_recurrent_scan__compressed_kv_cla__dense_activation_silu__decode_kernel(
    A_x: jax.Array,
    A_c_kv: jax.Array,
    A_w_q: jax.Array,
    A_w_uk: jax.Array,
    A_w_uv: jax.Array,
    A_w_o: jax.Array,
    B_x: jax.Array,
    B_w1: jax.Array,
    B_w2: jax.Array,
):
    del B_x
    B, Sq, M = A_x.shape
    _, S, DC = A_c_kv.shape
    _, H, D = A_w_q.shape
    F = B_w1.shape[1]
    assert (B, Sq, M, S, DC, H, D, F) == (1, 1, 512, 32768, 512, 32, 128, 1376)

    NB = 4
    G = 16
    NP = 128 // G

    KR, KA, KB = 48, 4, 17
    T = 1920
    NT = S // T
    SM = NT * T
    REM = S - SM
    NR = SM // (KA * KB * KR)
    DPT = T // (KA * KR)
    assert NR * KA * KB * KR == SM and DPT * KA * KR == T
    KW = 2
    WA, WB, WR = 5, 17, 192
    WM = WA * WB * WR
    WN = M * H
    GRP = (0, 4, 8, 12, 17)
    GW = 4

    CH, N1, AHEAD = 32, 6, 6
    RING = 2 * AHEAD
    NCH = N1 + F // CH
    R1 = N1 * CH
    TPI = 2

    WO_SPLIT = (0, 16 * D, 26 * D, 30 * D, 31 * D,
                31 * D + 80, 31 * D + 112, 32 * D)
    N_WO = len(WO_SPLIT) - 1
    N_MXU = 4
    WPI = -(-N_WO // KW)

    ckv2 = A_c_kv.reshape(S, DC)
    wq2 = A_w_q.reshape(WN, D)
    wuk2 = A_w_uk.reshape(WN, D)
    wuv2 = A_w_uv.reshape(WN, D)
    wo2 = A_w_o.reshape(H * D, M)
    w1t = B_w1.T

    def kernel(x_hbm, ckv_hbm, wq_hbm, wuk_hbm, wuv_hbm, wo_hbm, w1_hbm, w2_hbm,
               o_ref,
               x_v, ckv_v, rem_v, wq_v, wuk_v, wuv_v, wrest_v, wo_v, w1_v, w2_v,
               lhs_v, s_v, h_v, cb_v, af_v, mult_v, stage,
               sems, g_sems, kv_sems, wo_sems, h2s_sems, s2v_sems):
        c_x = pltpu.make_async_copy(x_hbm, x_v, sems.at[0])
        c_w1 = pltpu.make_async_copy(w1_hbm.at[pl.ds(R1, F - R1)],
                                     w1_v.at[pl.ds(R1, F - R1)], sems.at[1])
        c_rem = pltpu.make_async_copy(ckv_hbm.at[pl.ds(SM, REM)], rem_v,
                                      sems.at[2])
        ws = [(wq_hbm, wq_v), (wuk_hbm, wuk_v), (wuv_hbm, wuv_v)]
        NG = 4 * len(ws)

        def w_rest(g):
            return pltpu.make_async_copy(
                ws[g // 4][0].at[pl.ds(WM, WN - WM)], wrest_v.at[g // 4],
                sems.at[3 + g // 4])

        def start_group(g):
            src, dst = ws[g // 4]

            def body(b, carry):
                view = src.at[pl.ds(0, WM)].reshape(WA, WB, WR, D)
                pltpu.make_async_copy(view.at[:, b], dst.at[b],
                                      g_sems.at[g]).start()
                return carry

            lax.fori_loop(GRP[g % 4], GRP[g % 4 + 1], body, 0)
            if g % 4 == 0:
                w_rest(g).start()

        def wait_group(g):
            lo, hi = GRP[g % 4], GRP[g % 4 + 1]
            region = ws[g // 4][1].at[pl.ds(lo, hi - lo)]
            pltpu.make_async_copy(region, region, g_sems.at[g]).wait()
            if g % 4 == 0:
                w_rest(g).wait()

        def start_tile(i):
            def body(d, carry):
                view = ckv_hbm.at[pl.ds(0, SM)].reshape(NR, KA, KB, KR, DC)
                pltpu.make_async_copy(
                    view.at[d // KB, :, d % KB], ckv_v.at[pl.ds(d * KA, KA)],
                    kv_sems.at[i]).start()
                return carry

            lax.fori_loop(i * DPT, (i + 1) * DPT, body, 0)

        def tile_ref(i):
            return ckv_v.at[pl.ds(i * (T // KR), T // KR)]

        def wait_tile(i):
            pltpu.make_async_copy(tile_ref(i), tile_ref(i),
                                  kv_sems.at[i]).wait()

        c_wo = [
            pltpu.make_async_copy(wo_hbm.at[pl.ds(a, b - a)],
                                  wo_v.at[pl.ds(a, b - a)], wo_sems.at[k])
            for k, (a, b) in enumerate(zip(WO_SPLIT[:-1], WO_SPLIT[1:]))
        ]

        def step(g):
            wait_group(g)
            if g + GW < NG:
                start_group(g + GW)
            elif g == NG - 3:
                c_rem.start()
                start_tile(0)
            elif g == NG - 1:
                start_tile(1)

        def chunk(j):
            if isinstance(j, int):
                if j < N1:
                    return w1_hbm, w1_v, pl.ds(j * CH, CH)
                return w2_hbm, w2_v, pl.ds((j - N1) * CH, CH)
            return w2_hbm, w2_v, pl.ds(pl.multiple_of((j - N1) * CH, CH), CH)

        def h2s(j):
            src, _, rows = chunk(j)
            slot = j % RING
            return pltpu.make_async_copy(
                src.at[rows], stage.at[slot], h2s_sems.at[slot])

        def s2v(j):
            _, dst, rows = chunk(j)
            slot = j % RING
            return pltpu.make_async_copy(
                stage.at[slot], dst.at[rows], s2v_sems.at[slot])

        def tick(j):
            h2s(j).wait()
            s2v(j).start()
            if isinstance(j, int):
                if j + AHEAD < NCH:
                    if j >= AHEAD:
                        s2v(j - AHEAD).wait()
                    h2s(j + AHEAD).start()
            else:
                @pl.when(j + AHEAD < NCH)
                def _():
                    s2v(j - AHEAD).wait()
                    h2s(j + AHEAD).start()

        def slab(wi, c):
            spp = WR // H
            k = c // spp
            if k >= WA * WB:
                r = (c - WA * WB * spp) * H
                return wrest_v[wi, r:r + H, :]
            r = (c % spp) * H
            return ws[wi][1][k % WB, k // WB, r:r + H, :]

        def w_tiles(wi, n):
            return jnp.concatenate(
                [slab(wi, 128 * b + n * G + jj) for jj in range(G)
                 for b in range(NB)], axis=0)

        def head_mask(cols):
            r = lax.broadcasted_iota(jnp.int32, (H, cols), 0)
            c = lax.broadcasted_iota(jnp.int32, (H, cols), 1)
            return r == (c & (H - 1))

        def contract(a, wi):
            for b in range(NB):
                cb_v[b * H:(b + 1) * H, :] = a[:, b * 128:(b + 1) * 128]
            af_v[...] = cb_v[...].T
            mask = head_mask(128)
            out = jnp.zeros((H, D), _F32)
            for n in range(NP):
                lhs = jnp.concatenate(
                    [jnp.where(mask, af_v[pl.ds(n * G + jj, 1), :], 0.0)
                     .astype(_BF16) for jj in range(G)], axis=1)
                out = out + jnp.dot(lhs, w_tiles(wi, n),
                                    preferred_element_type=_F32)
            return out

        c_w1.start()
        h2s(0).start()
        start_group(0)
        for j in range(1, AHEAD):
            h2s(j).start()
        c_x.start()
        for g in range(1, GW):
            start_group(g)
        c_w1.wait()
        tick(0)
        for g in range(8):
            step(g)
            tick(g + 1)

        c_x.wait()
        x = x_v[0].astype(_F32)
        mu = jnp.mean(x, axis=-1, keepdims=True)
        xc = x - mu
        var = jnp.mean(xc * xc, axis=-1, keepdims=True)
        xn = xc * lax.rsqrt(var + 1e-5)
        lhs_v[:, 0:M] = jnp.broadcast_to(xn, (16, M)).astype(_BF16)
        xn16 = lhs_v[:, 0:M]
        q = contract(jnp.concatenate([xn16, xn16], axis=0).astype(_F32),
                     0).astype(_BF16)
        step(8)
        tick(9)

        for n in range(NP):
            t = lax.dot_general(q, w_tiles(1, n), _NT,
                                preferred_element_type=_F32)
            r = jnp.sum(jnp.where(head_mask(G * 128), t, 0.0), axis=0,
                        keepdims=True)
            for jj in range(G):
                af_v[pl.ds(n * G + jj, 1), :] = r[:, jj * 128:(jj + 1) * 128]
            if n == NP // 2 - 1:
                step(9)
                tick(10)
        z = af_v[...].T * (D ** -0.5)
        qa = jnp.concatenate(
            [z[b * H:(b + 1) * H] for b in range(NB)], axis=1).astype(_BF16)
        step(10)
        tick(11)
        step(11)
        tick(12)
        j_loop = 13
        assert j_loop - AHEAD >= N1 and j_loop + TPI * NT <= NCH

        h1 = lax.dot_general(xn16, w1_v[...], _NT, preferred_element_type=_F32)
        h_v[...] = _silu(h1).astype(_BF16)

        c_rem.wait()
        c0 = rem_v[...]
        s0 = lax.dot_general(qa, c0, _NT, preferred_element_type=_F32)
        m0 = jnp.max(s0, axis=-1, keepdims=True)
        p0 = jnp.exp(s0 - m0)
        init = (m0, jnp.sum(p0, axis=-1, keepdims=True),
                jnp.dot(p0.astype(_BF16), c0, preferred_element_type=_F32))

        def tile(i, carry):
            m, l, acc = carry
            wait_tile(i)

            @pl.when(i + KW < NT)
            def _():
                start_tile(i + KW)

            for k, cp in enumerate(c_wo):
                pl.when(i == NT - KW + k // WPI)(cp.start)
            for t in range(TPI):
                tick(i * TPI + t + j_loop)
            c = tile_ref(i)[...].reshape(T, DC)
            s = lax.dot_general(qa, c, _NT, preferred_element_type=_F32)
            m_new = jnp.maximum(m, jnp.max(s, axis=-1, keepdims=True))
            alpha = jnp.exp(m - m_new)
            p = jnp.exp(s - m_new)
            l = l * alpha + jnp.sum(p, axis=-1, keepdims=True)
            acc = acc * alpha + jnp.dot(p.astype(_BF16), c,
                                        preferred_element_type=_F32)
            return m_new, l, acc

        _, l, acc = lax.fori_loop(0, NT, tile, init)
        for j in range(j_loop + TPI * NT, NCH):
            tick(j)

        ctx = contract((acc * (1.0 / l)).astype(_BF16).astype(_F32),
                       2).astype(_BF16).astype(_F32)
        for h in range(H - 1):
            lhs_v[:, h * D:(h + 1) * D] = jnp.broadcast_to(
                ctx[h:h + 1], (16, D)).astype(_BF16)
        cb_v[...] = jnp.broadcast_to(ctx[H - 1:H], (D, D))
        af_v[...] = cb_v[...].T

        for k, (a, b) in enumerate(zip(WO_SPLIT[:-1], WO_SPLIT[1:])):
            if k == 1:
                for j in range(NCH - RING, NCH):
                    s2v(j).wait()
                g = _silu(jnp.dot(h_v[...], w2_v[...],
                                  preferred_element_type=_F32)[0:8])
                for bb in range(NB):
                    mult_v[:, bb * 128:(bb + 1) * 128] = (
                        af_v[...] * g[0:1, bb * 128:(bb + 1) * 128])
            c_wo[k].wait()
            if k < N_MXU:
                part = jnp.dot(lhs_v[:, a:b], wo_v[a:b, :],
                               preferred_element_type=_F32)[0:8]
                if k == 0:
                    s_v[...] = part
                elif k < N_MXU - 1:
                    s_v[...] += part
                else:
                    base = jnp.broadcast_to(x, (8, M)) + (s_v[...] + part) * g
                    row0 = lax.broadcasted_iota(jnp.int32, (8, M), 0) == 0
                    s_v[...] = jnp.where(row0, base, 0.0)
            else:
                r0 = a - (H - 1) * D
                prod = wo_v[a:b, :].astype(_F32) * mult_v[r0:r0 + b - a, :]
                parts = [s_v[...]] + [prod[r:r + 8] for r in range(0, b - a, 8)]
                while len(parts) > 1:
                    parts = [parts[i] + parts[i + 1] if i + 1 < len(parts)
                             else parts[i] for i in range(0, len(parts), 2)]
                if k < N_WO - 1:
                    s_v[...] = parts[0]
                else:
                    o_ref[0] = jnp.sum(parts[0], axis=0,
                                       keepdims=True).astype(o_ref.dtype)

    any_spec = pl.BlockSpec(memory_space=pl.ANY)
    return pl.pallas_call(
        kernel,
        out_shape=jax.ShapeDtypeStruct(A_x.shape, A_x.dtype),
        in_specs=[any_spec] * 8,
        out_specs=pl.BlockSpec(memory_space=pltpu.VMEM),
        scratch_shapes=[
            pltpu.VMEM(A_x.shape, _BF16),
            pltpu.VMEM((SM // KR, KR, DC), _BF16),
            pltpu.VMEM((REM, DC), _BF16),
            pltpu.VMEM((WB, WA, WR, D), _BF16),
            pltpu.VMEM((WB, WA, WR, D), _BF16),
            pltpu.VMEM((WB, WA, WR, D), _BF16),
            pltpu.VMEM((3, WN - WM, D), _BF16),
            pltpu.VMEM((H * D, M), _BF16),
            pltpu.VMEM((F, M), _BF16),
            pltpu.VMEM((F, M), _BF16),
            pltpu.VMEM((16, H * D), _BF16),
            pltpu.VMEM((8, M), _F32),
            pltpu.VMEM((16, F), _BF16),
            pltpu.VMEM((D, D), _F32),
            pltpu.VMEM((D, D), _F32),
            pltpu.VMEM((D, M), _F32),
            pltpu.SMEM((RING, CH, M), _BF16),
            pltpu.SemaphoreType.DMA((6,)),
            pltpu.SemaphoreType.DMA((12,)),
            pltpu.SemaphoreType.DMA((NT,)),
            pltpu.SemaphoreType.DMA((N_WO,)),
            pltpu.SemaphoreType.DMA((RING,)),
            pltpu.SemaphoreType.DMA((RING,)),
        ],
        compiler_params=_compiler_params(),
    )(A_x, ckv2, wq2, wuk2, wuv2, wo2, w1t, B_w2)
```

```python
import jax
import jax.numpy as jnp
from jax import lax
import jax.experimental.pallas as pl
import jax.experimental.pallas.tpu as pltpu

_NT = (((1,), (1,)), ((), ()))
_F32 = jnp.float32
_BF16 = jnp.bfloat16


def _silu(v):
    return v * (1.0 / (1.0 + jnp.exp(-v)))


def _compiler_params():
    limit = 100 * 1024 * 1024
    try:
        return pltpu.CompilerParams(vmem_limit_bytes=limit,
                                    disable_semaphore_checks=True)
    except TypeError:
        return pltpu.CompilerParams(vmem_limit_bytes=limit)


@jax.jit
def pallas_recurrent_scan__compressed_kv_cla__dense_activation_silu__decode_kernel(
    A_x: jax.Array,
    A_c_kv: jax.Array,
    A_w_q: jax.Array,
    A_w_uk: jax.Array,
    A_w_uv: jax.Array,
    A_w_o: jax.Array,
    B_x: jax.Array,
    B_w1: jax.Array,
    B_w2: jax.Array,
):
    del B_x
    B, Sq, M = A_x.shape
    _, S, DC = A_c_kv.shape
    _, H, D = A_w_q.shape
    F = B_w1.shape[1]
    assert (B, Sq, M, S, DC, H, D, F) == (1, 1, 512, 32768, 512, 32, 128, 1376)

    NB = 4
    G = 16
    NP = 128 // G

    KR, KA, KB = 48, 4, 17
    T = 1920
    NT = S // T
    SM = NT * T
    REM = S - SM
    NR = SM // (KA * KB * KR)
    DPT = T // (KA * KR)
    assert NR * KA * KB * KR == SM and DPT * KA * KR == T
    KW = 2
    WA, WB, WR = 5, 17, 192
    WM = WA * WB * WR
    WN = M * H
    GRP = (0, 4, 8, 12, 17)
    GW = 4

    CH, N1, AHEAD = 32, 6, 6
    RING = 2 * AHEAD
    NCH = N1 + F // CH
    R1 = N1 * CH
    TPI = 2

    WO_SPLIT = (0, 16 * D, 26 * D, 30 * D, 31 * D,
                31 * D + 80, 31 * D + 112, 32 * D)
    N_WO = len(WO_SPLIT) - 1
    N_MXU = 4
    WPI = -(-N_WO // KW)

    ckv2 = A_c_kv.reshape(S, DC)
    wq2 = A_w_q.reshape(WN, D)
    wuk2 = A_w_uk.reshape(WN, D)
    wuv2 = A_w_uv.reshape(WN, D)
    wo2 = A_w_o.reshape(H * D, M)
    w1t = B_w1.T

    def kernel(x_hbm, ckv_hbm, wq_hbm, wuk_hbm, wuv_hbm, wo_hbm, w1_hbm, w2_hbm,
               o_ref,
               x_v, ckv_v, rem_v, wq_v, wuk_v, wuv_v, wrest_v, wo_v, w1_v, w2_v,
               lhs_v, s_v, h_v, cb_v, af_v, mult_v, stage,
               sems, g_sems, kv_sems, wo_sems, h2s_sems, s2v_sems):
        c_x = pltpu.make_async_copy(x_hbm, x_v, sems.at[0])
        c_w1 = pltpu.make_async_copy(w1_hbm.at[pl.ds(R1, F - R1)],
                                     w1_v.at[pl.ds(R1, F - R1)], sems.at[1])
        c_rem = pltpu.make_async_copy(ckv_hbm.at[pl.ds(SM, REM)], rem_v,
                                      sems.at[2])
        ws = [(wq_hbm, wq_v), (wuk_hbm, wuk_v), (wuv_hbm, wuv_v)]
        NG = 4 * len(ws)

        def w_rest(g):
            return pltpu.make_async_copy(
                ws[g // 4][0].at[pl.ds(WM, WN - WM)], wrest_v.at[g // 4],
                sems.at[3 + g // 4])

        def start_group(g):
            src, dst = ws[g // 4]

            def body(b, carry):
                view = src.at[pl.ds(0, WM)].reshape(WA, WB, WR, D)
                pltpu.make_async_copy(view.at[:, b], dst.at[b],
                                      g_sems.at[g]).start()
                return carry

            lax.fori_loop(GRP[g % 4], GRP[g % 4 + 1], body, 0)
            if g % 4 == 0:
                w_rest(g).start()

        def wait_group(g):
            lo, hi = GRP[g % 4], GRP[g % 4 + 1]
            region = ws[g // 4][1].at[pl.ds(lo, hi - lo)]
            pltpu.make_async_copy(region, region, g_sems.at[g]).wait()
            if g % 4 == 0:
                w_rest(g).wait()

        def start_tile(i):
            def body(d, carry):
                view = ckv_hbm.at[pl.ds(0, SM)].reshape(NR, KA, KB, KR, DC)
                pltpu.make_async_copy(
                    view.at[d // KB, :, d % KB], ckv_v.at[pl.ds(d * KA, KA)],
                    kv_sems.at[i]).start()
                return carry

            lax.fori_loop(i * DPT, (i + 1) * DPT, body, 0)

        def tile_ref(i):
            return ckv_v.at[pl.ds(i * (T // KR), T // KR)]

        def wait_tile(i):
            pltpu.make_async_copy(tile_ref(i), tile_ref(i),
                                  kv_sems.at[i]).wait()

        c_wo = [
            pltpu.make_async_copy(wo_hbm.at[pl.ds(a, b - a)],
                                  wo_v.at[pl.ds(a, b - a)], wo_sems.at[k])
            for k, (a, b) in enumerate(zip(WO_SPLIT[:-1], WO_SPLIT[1:]))
        ]

        def step(g):
            wait_group(g)
            if g + GW < NG:
                start_group(g + GW)
            elif g == NG - 3:
                c_rem.start()
                start_tile(0)
            elif g == NG - 1:
                start_tile(1)

        def chunk(j):
            if isinstance(j, int):
                if j < N1:
                    return w1_hbm, w1_v, pl.ds(j * CH, CH)
                return w2_hbm, w2_v, pl.ds((j - N1) * CH, CH)
            return w2_hbm, w2_v, pl.ds(pl.multiple_of((j - N1) * CH, CH), CH)

        def h2s(j):
            src, _, rows = chunk(j)
            slot = j % RING
            return pltpu.make_async_copy(
                src.at[rows], stage.at[slot], h2s_sems.at[slot])

        def s2v(j):
            _, dst, rows = chunk(j)
            slot = j % RING
            return pltpu.make_async_copy(
                stage.at[slot], dst.at[rows], s2v_sems.at[slot])

        def tick(j):
            h2s(j).wait()
            s2v(j).start()
            if isinstance(j, int):
                if j + AHEAD < NCH:
                    if j >= AHEAD:
                        s2v(j - AHEAD).wait()
                    h2s(j + AHEAD).start()
            else:
                @pl.when(j + AHEAD < NCH)
                def _():
                    s2v(j - AHEAD).wait()
                    h2s(j + AHEAD).start()

        def slab(wi, c):
            spp = WR // H
            k = c // spp
            if k >= WA * WB:
                r = (c - WA * WB * spp) * H
                return wrest_v[wi, r:r + H, :]
            r = (c % spp) * H
            return ws[wi][1][k % WB, k // WB, r:r + H, :]

        def w_tiles(wi, n):
            return jnp.concatenate(
                [slab(wi, 128 * b + n * G + jj) for jj in range(G)
                 for b in range(NB)], axis=0)

        def head_mask(cols):
            r = lax.broadcasted_iota(jnp.int32, (H, cols), 0)
            c = lax.broadcasted_iota(jnp.int32, (H, cols), 1)
            return r == (c & (H - 1))

        def contract(a, wi):
            for b in range(NB):
                cb_v[b * H:(b + 1) * H, :] = a[:, b * 128:(b + 1) * 128]
            af_v[...] = cb_v[...].T
            mask = head_mask(128)
            out = jnp.zeros((H, D), _F32)
            for n in range(NP):
                lhs = jnp.concatenate(
                    [jnp.where(mask, af_v[pl.ds(n * G + jj, 1), :], 0.0)
                     .astype(_BF16) for jj in range(G)], axis=1)
                out = out + jnp.dot(lhs, w_tiles(wi, n),
                                    preferred_element_type=_F32)
            return out

        c_w1.start()
        h2s(0).start()
        start_group(0)
        for j in range(1, AHEAD):
            h2s(j).start()
        c_x.start()
        for g in range(1, GW):
            start_group(g)
        tick(0)
        c_w1.wait()
        tick(1)
        for g in range(8):
            step(g)
            tick(g + 2)

        c_x.wait()
        x = x_v[0].astype(_F32)
        mu = jnp.mean(x, axis=-1, keepdims=True)
        xc = x - mu
        var = jnp.mean(xc * xc, axis=-1, keepdims=True)
        xn = xc * lax.rsqrt(var + 1e-5)
        lhs_v[:, 0:M] = jnp.broadcast_to(xn, (16, M)).astype(_BF16)
        xn16 = lhs_v[:, 0:M]
        q = contract(jnp.concatenate([xn16, xn16], axis=0).astype(_F32),
                     0).astype(_BF16)
        step(8)
        tick(10)

        for n in range(NP):
            t = lax.dot_general(q, w_tiles(1, n), _NT,
                                preferred_element_type=_F32)
            r = jnp.sum(jnp.where(head_mask(G * 128), t, 0.0), axis=0,
                        keepdims=True)
            for jj in range(G):
                af_v[pl.ds(n * G + jj, 1), :] = r[:, jj * 128:(jj + 1) * 128]
            if n == NP // 2 - 1:
                step(9)
                tick(11)
        z = af_v[...].T * (D ** -0.5)
        qa = jnp.concatenate(
            [z[b * H:(b + 1) * H] for b in range(NB)], axis=1).astype(_BF16)
        step(10)
        tick(12)
        step(11)
        tick(13)
        j_loop = 14
        assert j_loop - AHEAD >= N1 and j_loop + TPI * NT <= NCH

        h1 = lax.dot_general(xn16, w1_v[...], _NT, preferred_element_type=_F32)
        h_v[...] = _silu(h1).astype(_BF16)

        c_rem.wait()
        c0 = rem_v[...]
        s0 = lax.dot_general(qa, c0, _NT, preferred_element_type=_F32)
        m0 = jnp.max(s0, axis=-1, keepdims=True)
        p0 = jnp.exp(s0 - m0)
        init = (m0, jnp.sum(p0, axis=-1, keepdims=True),
                jnp.dot(p0.astype(_BF16), c0, preferred_element_type=_F32))

        def tile(i, carry):
            m, l, acc = carry
            wait_tile(i)

            @pl.when(i + KW < NT)
            def _():
                start_tile(i + KW)

            for k, cp in enumerate(c_wo):
                pl.when(i == NT - KW + k // WPI)(cp.start)
            for t in range(TPI):
                tick(i * TPI + t + j_loop)
            c = tile_ref(i)[...].reshape(T, DC)
            s = lax.dot_general(qa, c, _NT, preferred_element_type=_F32)
            m_new = jnp.maximum(m, jnp.max(s, axis=-1, keepdims=True))
            alpha = jnp.exp(m - m_new)
            p = jnp.exp(s - m_new)
            l = l * alpha + jnp.sum(p, axis=-1, keepdims=True)
            acc = acc * alpha + jnp.dot(p.astype(_BF16), c,
                                        preferred_element_type=_F32)
            return m_new, l, acc

        _, l, acc = lax.fori_loop(0, NT, tile, init)
        for j in range(j_loop + TPI * NT, NCH):
            tick(j)

        ctx = contract((acc * (1.0 / l)).astype(_BF16).astype(_F32),
                       2).astype(_BF16).astype(_F32)
        for h in range(H - 1):
            lhs_v[:, h * D:(h + 1) * D] = jnp.broadcast_to(
                ctx[h:h + 1], (16, D)).astype(_BF16)
        cb_v[...] = jnp.broadcast_to(ctx[H - 1:H], (D, D))
        af_v[...] = cb_v[...].T

        for k, (a, b) in enumerate(zip(WO_SPLIT[:-1], WO_SPLIT[1:])):
            if k == 1:
                for j in range(NCH - RING, NCH):
                    s2v(j).wait()
                g = _silu(jnp.dot(h_v[...], w2_v[...],
                                  preferred_element_type=_F32)[0:8])
                for bb in range(NB):
                    mult_v[:, bb * 128:(bb + 1) * 128] = (
                        af_v[...] * g[0:1, bb * 128:(bb + 1) * 128])
            c_wo[k].wait()
            if k < N_MXU:
                part = jnp.dot(lhs_v[:, a:b], wo_v[a:b, :],
                               preferred_element_type=_F32)[0:8]
                if k == 0:
                    s_v[...] = part
                elif k < N_MXU - 1:
                    s_v[...] += part
                else:
                    base = jnp.broadcast_to(x, (8, M)) + (s_v[...] + part) * g
                    row0 = lax.broadcasted_iota(jnp.int32, (8, M), 0) == 0
                    s_v[...] = jnp.where(row0, base, 0.0)
            else:
                r0 = a - (H - 1) * D
                prod = wo_v[a:b, :].astype(_F32) * mult_v[r0:r0 + b - a, :]
                parts = [s_v[...]] + [prod[r:r + 8] for r in range(0, b - a, 8)]
                while len(parts) > 1:
                    parts = [parts[i] + parts[i + 1] if i + 1 < len(parts)
                             else parts[i] for i in range(0, len(parts), 2)]
                if k < N_WO - 1:
                    s_v[...] = parts[0]
                else:
                    o_ref[0] = jnp.sum(parts[0], axis=0,
                                       keepdims=True).astype(o_ref.dtype)

    any_spec = pl.BlockSpec(memory_space=pl.ANY)
    return pl.pallas_call(
        kernel,
        out_shape=jax.ShapeDtypeStruct(A_x.shape, A_x.dtype),
        in_specs=[any_spec] * 8,
        out_specs=pl.BlockSpec(memory_space=pltpu.VMEM),
        scratch_shapes=[
            pltpu.VMEM(A_x.shape, _BF16),
            pltpu.VMEM((SM // KR, KR, DC), _BF16),
            pltpu.VMEM((REM, DC), _BF16),
            pltpu.VMEM((WB, WA, WR, D), _BF16),
            pltpu.VMEM((WB, WA, WR, D), _BF16),
            pltpu.VMEM((WB, WA, WR, D), _BF16),
            pltpu.VMEM((3, WN - WM, D), _BF16),
            pltpu.VMEM((H * D, M), _BF16),
            pltpu.VMEM((F, M), _BF16),
            pltpu.VMEM((F, M), _BF16),
            pltpu.VMEM((16, H * D), _BF16),
            pltpu.VMEM((8, M), _F32),
            pltpu.VMEM((16, F), _BF16),
            pltpu.VMEM((D, D), _F32),
            pltpu.VMEM((D, D), _F32),
            pltpu.VMEM((D, M), _F32),
            pltpu.SMEM((RING, CH, M), _BF16),
            pltpu.SemaphoreType.DMA((6,)),
            pltpu.SemaphoreType.DMA((12,)),
            pltpu.SemaphoreType.DMA((NT,)),
            pltpu.SemaphoreType.DMA((N_WO,)),
            pltpu.SemaphoreType.DMA((RING,)),
            pltpu.SemaphoreType.DMA((RING,)),
        ],
        compiler_params=_compiler_params(),
    )(A_x, ckv2, wq2, wuk2, wuv2, wo2, w1t, B_w2)
```

```python
import jax
import jax.numpy as jnp
from jax import lax
import jax.experimental.pallas as pl
import jax.experimental.pallas.tpu as pltpu

_NT = (((1,), (1,)), ((), ()))
_F32 = jnp.float32
_BF16 = jnp.bfloat16


def _silu(v):
    return v * (1.0 / (1.0 + jnp.exp(-v)))


def _compiler_params():
    limit = 100 * 1024 * 1024
    try:
        return pltpu.CompilerParams(vmem_limit_bytes=limit,
                                    disable_semaphore_checks=True)
    except TypeError:
        return pltpu.CompilerParams(vmem_limit_bytes=limit)


@jax.jit
def pallas_recurrent_scan__compressed_kv_cla__dense_activation_silu__decode_kernel(
    A_x: jax.Array,
    A_c_kv: jax.Array,
    A_w_q: jax.Array,
    A_w_uk: jax.Array,
    A_w_uv: jax.Array,
    A_w_o: jax.Array,
    B_x: jax.Array,
    B_w1: jax.Array,
    B_w2: jax.Array,
):
    del B_x
    B, Sq, M = A_x.shape
    _, S, DC = A_c_kv.shape
    _, H, D = A_w_q.shape
    F = B_w1.shape[1]
    assert (B, Sq, M, S, DC, H, D, F) == (1, 1, 512, 32768, 512, 32, 128, 1376)

    NB = 4
    G = 16
    NP = 128 // G

    KR, KA, KB = 48, 4, 17
    T = 1920
    NT = S // T
    SM = NT * T
    REM = S - SM
    NR = SM // (KA * KB * KR)
    DPT = T // (KA * KR)
    assert NR * KA * KB * KR == SM and DPT * KA * KR == T
    KW = 2
    WA, WB, WR = 5, 17, 192
    WM = WA * WB * WR
    WN = M * H
    GRP = (0, 4, 8, 12, 17)
    GW = 4

    CH, N1, AHEAD = 32, 6, 4
    RING = 2 * AHEAD
    NCH = N1 + F // CH
    R1 = N1 * CH
    G1 = 1152

    WO_SPLIT = (0, 16 * D, 24 * D, 28 * D, 30 * D, 31 * D,
                31 * D + 80, 31 * D + 112, 32 * D)
    N_WO = len(WO_SPLIT) - 1
    N_MXU = 4
    NV = H - WO_SPLIT[N_MXU] // D
    WPI = -(-N_WO // KW)

    ckv2 = A_c_kv.reshape(S, DC)
    wq2 = A_w_q.reshape(WN, D)
    wuk2 = A_w_uk.reshape(WN, D)
    wuv2 = A_w_uv.reshape(WN, D)
    wo2 = A_w_o.reshape(H * D, M)
    w1t = B_w1.T

    def kernel(x_hbm, ckv_hbm, wq_hbm, wuk_hbm, wuv_hbm, wo_hbm, w1_hbm, w2_hbm,
               o_ref,
               x_v, ckv_v, rem_v, wq_v, wuk_v, wuv_v, wrest_v, wo_v, w1_v, w2_v,
               lhs_v, s_v, g_v, h_v, acc_v, cb_v, af_v, col_v, mult_v, stage,
               sems, g_sems, kv_sems, wo_sems, h2s_sems, s2v_sems):
        c_x = pltpu.make_async_copy(x_hbm, x_v, sems.at[0])
        c_w1 = pltpu.make_async_copy(w1_hbm.at[pl.ds(R1, F - R1)],
                                     w1_v.at[pl.ds(R1, F - R1)], sems.at[1])
        c_rem = pltpu.make_async_copy(ckv_hbm.at[pl.ds(SM, REM)], rem_v,
                                      sems.at[2])
        ws = [(wq_hbm, wq_v), (wuk_hbm, wuk_v), (wuv_hbm, wuv_v)]
        NG = 4 * len(ws)

        def w_rest(g):
            return pltpu.make_async_copy(
                ws[g // 4][0].at[pl.ds(WM, WN - WM)], wrest_v.at[g // 4],
                sems.at[3 + g // 4])

        def start_group(g):
            src, dst = ws[g // 4]

            def body(b, carry):
                view = src.at[pl.ds(0, WM)].reshape(WA, WB, WR, D)
                pltpu.make_async_copy(view.at[:, b], dst.at[b],
                                      g_sems.at[g]).start()
                return carry

            lax.fori_loop(GRP[g % 4], GRP[g % 4 + 1], body, 0)
            if g % 4 == 0:
                w_rest(g).start()

        def wait_group(g):
            lo, hi = GRP[g % 4], GRP[g % 4 + 1]
            region = ws[g // 4][1].at[pl.ds(lo, hi - lo)]
            pltpu.make_async_copy(region, region, g_sems.at[g]).wait()
            if g % 4 == 0:
                w_rest(g).wait()

        def start_tile(i):
            def body(dd, carry):
                d = i * DPT + dd
                view = ckv_hbm.at[pl.ds(0, SM)].reshape(NR, KA, KB, KR, DC)
                pltpu.make_async_copy(
                    view.at[d // KB, :, d % KB], ckv_v.at[pl.ds(d * KA, KA)],
                    kv_sems.at[i]).start()
                return carry

            lax.fori_loop(0, DPT, body, 0)

        def tile_ref(i):
            return ckv_v.at[pl.ds(i * (T // KR), T // KR)]

        def wait_tile(i):
            pltpu.make_async_copy(tile_ref(i), tile_ref(i),
                                  kv_sems.at[i]).wait()

        c_wo = [
            pltpu.make_async_copy(wo_hbm.at[pl.ds(a, b - a)],
                                  wo_v.at[pl.ds(a, b - a)], wo_sems.at[k])
            for k, (a, b) in enumerate(zip(WO_SPLIT[:-1], WO_SPLIT[1:]))
        ]

        def step(g):
            wait_group(g)
            if g + GW < NG:
                start_group(g + GW)
            elif g == NG - 3:
                c_rem.start()
                start_tile(0)
            elif g == NG - 1:
                start_tile(1)

        def chunk(j):
            if isinstance(j, int):
                if j < N1:
                    return w1_hbm, w1_v, pl.ds(j * CH, CH)
                return w2_hbm, w2_v, pl.ds((j - N1) * CH, CH)
            return w2_hbm, w2_v, pl.ds(pl.multiple_of((j - N1) * CH, CH), CH)

        def h2s(j):
            src, _, rows = chunk(j)
            slot = j % RING
            return pltpu.make_async_copy(
                src.at[rows], stage.at[slot], h2s_sems.at[slot])

        def s2v(j):
            _, dst, rows = chunk(j)
            slot = j % RING
            return pltpu.make_async_copy(
                stage.at[slot], dst.at[rows], s2v_sems.at[slot])

        def tick(j):
            h2s(j).wait()
            s2v(j).start()
            if isinstance(j, int):
                if j + AHEAD < NCH:
                    if j >= AHEAD:
                        s2v(j - AHEAD).wait()
                    h2s(j + AHEAD).start()
            else:
                @pl.when(j + AHEAD < NCH)
                def _():
                    s2v(j - AHEAD).wait()
                    h2s(j + AHEAD).start()

        def slab(wi, c):
            spp = WR // H
            k = c // spp
            if k >= WA * WB:
                r = (c - WA * WB * spp) * H
                return wrest_v[wi, r:r + H, :]
            r = (c % spp) * H
            return ws[wi][1][k % WB, k // WB, r:r + H, :]

        def w_tiles(wi, n):
            return jnp.concatenate(
                [slab(wi, 128 * b + n * G + jj) for jj in range(G)
                 for b in range(NB)], axis=0)

        def head_mask(cols):
            r = lax.broadcasted_iota(jnp.int32, (H, cols), 0)
            c = lax.broadcasted_iota(jnp.int32, (H, cols), 1)
            return r == (c & (H - 1))

        def contract(a, wi):
            for b in range(NB):
                cb_v[b * H:(b + 1) * H, :] = a[:, b * 128:(b + 1) * 128]
            af_v[...] = cb_v[...].T
            mask = head_mask(128)
            out = jnp.zeros((H, D), _F32)
            for n in range(NP):
                lhs = jnp.concatenate(
                    [jnp.where(mask, af_v[pl.ds(n * G + jj, 1), :], 0.0)
                     .astype(_BF16) for jj in range(G)], axis=1)
                out = out + jnp.dot(lhs, w_tiles(wi, n),
                                    preferred_element_type=_F32)
            return out

        c_w1.start()
        h2s(0).start()
        start_group(0)
        for j in range(1, AHEAD):
            h2s(j).start()
        c_x.start()
        for g in range(1, GW):
            start_group(g)
        tick(0)
        c_w1.wait()
        tick(1)
        for g in range(8):
            step(g)
            tick(g + 2)

        c_x.wait()
        x = x_v[0].astype(_F32)
        mu = jnp.mean(x, axis=-1, keepdims=True)
        xc = x - mu
        var = jnp.mean(xc * xc, axis=-1, keepdims=True)
        xn = xc * lax.rsqrt(var + 1e-5)
        lhs_v[:, 0:M] = jnp.broadcast_to(xn, (16, M)).astype(_BF16)
        xn16 = lhs_v[:, 0:M]
        q = contract(jnp.concatenate([xn16, xn16], axis=0).astype(_F32),
                     0).astype(_BF16)
        step(8)
        tick(10)

        for n in range(NP):
            t = lax.dot_general(q, w_tiles(1, n), _NT,
                                preferred_element_type=_F32)
            r = jnp.sum(jnp.where(head_mask(G * 128), t, 0.0), axis=0,
                        keepdims=True)
            for jj in range(G):
                af_v[pl.ds(n * G + jj, 1), :] = r[:, jj * 128:(jj + 1) * 128]
            if n == NP // 2 - 1:
                step(9)
                tick(11)
        z = af_v[...].T * (D ** -0.5)
        qa = jnp.concatenate(
            [z[b * H:(b + 1) * H] for b in range(NB)], axis=1).astype(_BF16)
        step(10)
        tick(12)
        step(11)
        tick(13)
        j_loop = 14
        assert j_loop - AHEAD >= N1 and j_loop + 2 * NT <= NCH

        h1 = lax.dot_general(xn16, w1_v[...], _NT, preferred_element_type=_F32)
        h_v[...] = _silu(h1).astype(_BF16)

        c_rem.wait()
        c0 = rem_v[...]
        s0 = lax.dot_general(qa, c0, _NT, preferred_element_type=_F32)
        m0 = jnp.max(s0, axis=-1, keepdims=True)
        p0 = jnp.exp(s0 - m0)
        init = (m0, jnp.sum(p0, axis=-1, keepdims=True),
                jnp.dot(p0.astype(_BF16), c0, preferred_element_type=_F32))

        def tile(i, carry):
            m, l, acc = carry
            wait_tile(i)

            @pl.when(i + KW < NT)
            def _():
                start_tile(i + KW)

            for k, cp in enumerate(c_wo):
                pl.when(i == NT - KW + k // WPI)(cp.start)
            tick(2 * i + j_loop)
            c = tile_ref(i)[...].reshape(T, DC)
            s = lax.dot_general(qa, c, _NT, preferred_element_type=_F32)
            m_new = jnp.maximum(m, jnp.max(s, axis=-1, keepdims=True))
            alpha = jnp.exp(m - m_new)
            p = jnp.exp(s - m_new)
            l = l * alpha + jnp.sum(p, axis=-1, keepdims=True)
            acc_v[...] = acc * alpha + jnp.dot(p.astype(_BF16), c,
                                               preferred_element_type=_F32)
            tick(2 * i + 1 + j_loop)
            return m_new, l, acc_v[...]

        _, l, acc = lax.fori_loop(0, NT, tile, init)

        ctx = contract((acc * (1.0 / l)).astype(_BF16).astype(_F32),
                       2).astype(_BF16).astype(_F32)
        for h in range(H - NV):
            lhs_v[:, h * D:(h + 1) * D] = jnp.broadcast_to(
                ctx[h:h + 1], (16, D)).astype(_BF16)
        for v in range(NV):
            cb_v[...] = jnp.broadcast_to(ctx[H - NV + v:H - NV + v + 1], (D, D))
            col_v[v * D:(v + 1) * D, :] = cb_v[...].T
        for j in range(j_loop + 2 * NT, NCH):
            tick(j)

        n_early = N1 + G1 // CH
        for j in range(NCH - RING, n_early):
            s2v(j).wait()
        g_v[...] = jnp.dot(h_v[:, 0:G1], w2_v[0:G1, :],
                           preferred_element_type=_F32)[0:8]

        for k, (a, b) in enumerate(zip(WO_SPLIT[:-1], WO_SPLIT[1:])):
            if k == 2:
                for j in range(max(n_early, NCH - RING), NCH):
                    s2v(j).wait()
                g = _silu(g_v[...] + jnp.dot(h_v[:, G1:F], w2_v[G1:F, :],
                                             preferred_element_type=_F32)[0:8])
                for bb in range(NB):
                    mult_v[:, bb * 128:(bb + 1) * 128] = (
                        col_v[...] * g[0:1, bb * 128:(bb + 1) * 128])
            c_wo[k].wait()
            if k < N_MXU:
                part = jnp.dot(lhs_v[:, a:b], wo_v[a:b, :],
                               preferred_element_type=_F32)[0:8]
                if k == 0:
                    s_v[...] = part
                elif k < N_MXU - 1:
                    s_v[...] += part
                else:
                    base = jnp.broadcast_to(x, (8, M)) + (s_v[...] + part) * g
                    row0 = lax.broadcasted_iota(jnp.int32, (8, M), 0) == 0
                    s_v[...] = jnp.where(row0, base, 0.0)
            else:
                r0 = a - (H - NV) * D
                prod = wo_v[a:b, :].astype(_F32) * mult_v[r0:r0 + b - a, :]
                parts = [s_v[...]] + [prod[r:r + 8] for r in range(0, b - a, 8)]
                while len(parts) > 1:
                    parts = [parts[i] + parts[i + 1] if i + 1 < len(parts)
                             else parts[i] for i in range(0, len(parts), 2)]
                if k < N_WO - 1:
                    s_v[...] = parts[0]
                else:
                    o_ref[0] = jnp.sum(parts[0], axis=0,
                                       keepdims=True).astype(o_ref.dtype)

    any_spec = pl.BlockSpec(memory_space=pl.ANY)
    return pl.pallas_call(
        kernel,
        out_shape=jax.ShapeDtypeStruct(A_x.shape, A_x.dtype),
        in_specs=[any_spec] * 8,
        out_specs=pl.BlockSpec(memory_space=pltpu.VMEM),
        scratch_shapes=[
            pltpu.VMEM(A_x.shape, _BF16),
            pltpu.VMEM((SM // KR, KR, DC), _BF16),
            pltpu.VMEM((REM, DC), _BF16),
            pltpu.VMEM((WB, WA, WR, D), _BF16),
            pltpu.VMEM((WB, WA, WR, D), _BF16),
            pltpu.VMEM((WB, WA, WR, D), _BF16),
            pltpu.VMEM((3, WN - WM, D), _BF16),
            pltpu.VMEM((H * D, M), _BF16),
            pltpu.VMEM((F, M), _BF16),
            pltpu.VMEM((F, M), _BF16),
            pltpu.VMEM((16, H * D), _BF16),
            pltpu.VMEM((8, M), _F32),
            pltpu.VMEM((8, M), _F32),
            pltpu.VMEM((16, F), _BF16),
            pltpu.VMEM((H, DC), _F32),
            pltpu.VMEM((D, D), _F32),
            pltpu.VMEM((D, D), _F32),
            pltpu.VMEM((NV * D, D), _F32),
            pltpu.VMEM((NV * D, M), _F32),
            pltpu.SMEM((RING, CH, M), _BF16),
            pltpu.SemaphoreType.DMA((6,)),
            pltpu.SemaphoreType.DMA((12,)),
            pltpu.SemaphoreType.DMA((NT,)),
            pltpu.SemaphoreType.DMA((N_WO,)),
            pltpu.SemaphoreType.DMA((RING,)),
            pltpu.SemaphoreType.DMA((RING,)),
        ],
        compiler_params=_compiler_params(),
    )(A_x, ckv2, wq2, wuk2, wuv2, wo2, w1t, B_w2)
```

```python
import jax
import jax.numpy as jnp
from jax import lax
import jax.experimental.pallas as pl
import jax.experimental.pallas.tpu as pltpu

_NT = (((1,), (1,)), ((), ()))
_F32 = jnp.float32
_BF16 = jnp.bfloat16


def _silu(v):
    return v * (1.0 / (1.0 + jnp.exp(-v)))


def _compiler_params():
    limit = 100 * 1024 * 1024
    try:
        return pltpu.CompilerParams(vmem_limit_bytes=limit,
                                    disable_semaphore_checks=True)
    except TypeError:
        return pltpu.CompilerParams(vmem_limit_bytes=limit)


@jax.jit
def pallas_recurrent_scan__compressed_kv_cla__dense_activation_silu__decode_kernel(
    A_x: jax.Array,
    A_c_kv: jax.Array,
    A_w_q: jax.Array,
    A_w_uk: jax.Array,
    A_w_uv: jax.Array,
    A_w_o: jax.Array,
    B_x: jax.Array,
    B_w1: jax.Array,
    B_w2: jax.Array,
):
    del B_x
    B, Sq, M = A_x.shape
    _, S, DC = A_c_kv.shape
    _, H, D = A_w_q.shape
    F = B_w1.shape[1]
    assert (B, Sq, M, S, DC, H, D, F) == (1, 1, 512, 32768, 512, 32, 128, 1376)

    NB = 4
    G = 16
    NP = 128 // G

    KR, KA = 48, 4
    KQ = S // KA
    T = 1920
    NT = S // T
    SM = NT * T
    REM = S - SM
    DPT = T // (KA * KR)
    assert DPT * KA * KR == T
    KW = 2
    LW = 128 * H
    WR = 192
    WB = LW // WR
    GRP = (0, 5, 10, 15, WB)
    GW = 3

    CH, N1, AHEAD = 32, 6, 4
    RING = 2 * AHEAD
    NCH = N1 + F // CH
    R1 = N1 * CH
    G1 = 1152

    WO_SPLIT = (0, 16 * D, 24 * D, 28 * D, 30 * D, 31 * D,
                31 * D + 80, 31 * D + 112, 32 * D)
    N_WO = len(WO_SPLIT) - 1
    N_MXU = 4
    NV = H - WO_SPLIT[N_MXU] // D
    WPI = -(-N_WO // KW)

    ckv2 = A_c_kv.reshape(KA, KQ, DC)
    wq2 = A_w_q.reshape(NB, LW, D)
    wuk2 = A_w_uk.reshape(NB, LW, D)
    wuv2 = A_w_uv.reshape(NB, LW, D)
    wo2 = A_w_o.reshape(H * D, M)
    w1t = B_w1.T

    def kernel(x_hbm, ckv_hbm, wq_hbm, wuk_hbm, wuv_hbm, wo_hbm, w1_hbm, w2_hbm,
               o_ref,
               x_v, ckv_v, rem_v, wq_v, wuk_v, wuv_v, wo_v, w1_v, w2_v,
               lhs_v, s_v, g_v, h_v, acc_v, cb_v, af_v, col_v, mult_v, stage,
               sems, g_sems, kv_sems, wo_sems, h2s_sems, s2v_sems):
        c_x = pltpu.make_async_copy(x_hbm, x_v, sems.at[0])
        c_w1 = pltpu.make_async_copy(w1_hbm.at[pl.ds(R1, F - R1)],
                                     w1_v.at[pl.ds(R1, F - R1)], sems.at[1])
        c_rem = pltpu.make_async_copy(
            ckv_hbm.at[:, pl.ds(SM // KA, REM // KA)], rem_v, sems.at[2])
        ws = [(wq_hbm, wq_v), (wuk_hbm, wuk_v), (wuv_hbm, wuv_v)]
        NG = 4 * len(ws)

        def start_group(g):
            src, dst = ws[g // 4]

            def body(b, carry):
                rows = pl.ds(pl.multiple_of(b * WR, WR), WR)
                pltpu.make_async_copy(src.at[:, rows], dst.at[:, rows],
                                      g_sems.at[g]).start()
                return carry

            lax.fori_loop(GRP[g % 4], GRP[g % 4 + 1], body, 0)
            if g % 4 == 3:
                rows = pl.ds(WB * WR, LW - WB * WR)
                pltpu.make_async_copy(src.at[:, rows], dst.at[:, rows],
                                      g_sems.at[g]).start()

        def wait_group(g):
            lo = GRP[g % 4] * WR
            hi = LW if g % 4 == 3 else GRP[g % 4 + 1] * WR
            region = ws[g // 4][1].at[:, pl.ds(lo, hi - lo)]
            pltpu.make_async_copy(region, region, g_sems.at[g]).wait()

        def start_tile(i):
            def body(dd, carry):
                d = i * DPT + dd
                pltpu.make_async_copy(
                    ckv_hbm.at[:, pl.ds(pl.multiple_of(d * KR, KR), KR)],
                    ckv_v.at[pl.ds(d * KA, KA)], kv_sems.at[i]).start()
                return carry

            lax.fori_loop(0, DPT, body, 0)

        def tile_ref(i):
            return ckv_v.at[pl.ds(i * (T // KR), T // KR)]

        def wait_tile(i):
            pltpu.make_async_copy(tile_ref(i), tile_ref(i),
                                  kv_sems.at[i]).wait()

        c_wo = [
            pltpu.make_async_copy(wo_hbm.at[pl.ds(a, b - a)],
                                  wo_v.at[pl.ds(a, b - a)], wo_sems.at[k])
            for k, (a, b) in enumerate(zip(WO_SPLIT[:-1], WO_SPLIT[1:]))
        ]

        def step(g):
            wait_group(g)
            if g + GW < NG:
                start_group(g + GW)
            elif g == NG - 3:
                c_rem.start()
                start_tile(0)
            elif g == NG - 1:
                start_tile(1)

        def chunk(j):
            if isinstance(j, int):
                if j < N1:
                    return w1_hbm, w1_v, pl.ds(j * CH, CH)
                return w2_hbm, w2_v, pl.ds((j - N1) * CH, CH)
            return w2_hbm, w2_v, pl.ds(pl.multiple_of((j - N1) * CH, CH), CH)

        def h2s(j):
            src, _, rows = chunk(j)
            slot = j % RING
            return pltpu.make_async_copy(
                src.at[rows], stage.at[slot], h2s_sems.at[slot])

        def s2v(j):
            _, dst, rows = chunk(j)
            slot = j % RING
            return pltpu.make_async_copy(
                stage.at[slot], dst.at[rows], s2v_sems.at[slot])

        def tick(j):
            h2s(j).wait()
            s2v(j).start()
            if isinstance(j, int):
                if j + AHEAD < NCH:
                    if j >= AHEAD:
                        s2v(j - AHEAD).wait()
                    h2s(j + AHEAD).start()
            else:
                @pl.when(j + AHEAD < NCH)
                def _():
                    s2v(j - AHEAD).wait()
                    h2s(j + AHEAD).start()

        def w_tiles(wi, n):
            w = ws[wi][1]
            return jnp.concatenate(
                [w[b, (n * G + jj) * H:(n * G + jj + 1) * H, :]
                 for jj in range(G) for b in range(NB)], axis=0)

        def head_mask(cols):
            r = lax.broadcasted_iota(jnp.int32, (H, cols), 0)
            c = lax.broadcasted_iota(jnp.int32, (H, cols), 1)
            return r == (c & (H - 1))

        def contract(a, wi):
            for b in range(NB):
                cb_v[b * H:(b + 1) * H, :] = a[:, b * 128:(b + 1) * 128]
            af_v[...] = cb_v[...].T
            mask = head_mask(128)
            out = jnp.zeros((H, D), _F32)
            for n in range(NP):
                lhs = jnp.concatenate(
                    [jnp.where(mask, af_v[pl.ds(n * G + jj, 1), :], 0.0)
                     .astype(_BF16) for jj in range(G)], axis=1)
                out = out + jnp.dot(lhs, w_tiles(wi, n),
                                    preferred_element_type=_F32)
            return out

        c_w1.start()
        h2s(0).start()
        start_group(0)
        for j in range(1, AHEAD):
            h2s(j).start()
        c_x.start()
        for g in range(1, GW):
            start_group(g)
        tick(0)
        c_w1.wait()
        tick(1)
        for g in range(8):
            step(g)
            tick(g + 2)

        c_x.wait()
        x = x_v[0].astype(_F32)
        mu = jnp.mean(x, axis=-1, keepdims=True)
        xc = x - mu
        var = jnp.mean(xc * xc, axis=-1, keepdims=True)
        xn = xc * lax.rsqrt(var + 1e-5)
        lhs_v[:, 0:M] = jnp.broadcast_to(xn, (16, M)).astype(_BF16)
        xn16 = lhs_v[:, 0:M]
        q = contract(jnp.concatenate([xn16, xn16], axis=0).astype(_F32),
                     0).astype(_BF16)
        step(8)
        tick(10)

        for n in range(NP):
            t = lax.dot_general(q, w_tiles(1, n), _NT,
                                preferred_element_type=_F32)
            r = jnp.sum(jnp.where(head_mask(G * 128), t, 0.0), axis=0,
                        keepdims=True)
            for jj in range(G):
                af_v[pl.ds(n * G + jj, 1), :] = r[:, jj * 128:(jj + 1) * 128]
            if n == NP // 2 - 1:
                step(9)
                tick(11)
        z = af_v[...].T * (D ** -0.5)
        qa = jnp.concatenate(
            [z[b * H:(b + 1) * H] for b in range(NB)], axis=1).astype(_BF16)
        step(10)
        tick(12)
        step(11)
        tick(13)
        j_loop = 14
        assert j_loop - AHEAD >= N1 and j_loop + 2 * NT <= NCH

        h1 = lax.dot_general(xn16, w1_v[...], _NT, preferred_element_type=_F32)
        h_v[...] = _silu(h1).astype(_BF16)

        c_rem.wait()
        c0 = rem_v[...].reshape(REM, DC)
        s0 = lax.dot_general(qa, c0, _NT, preferred_element_type=_F32)
        m0 = jnp.max(s0, axis=-1, keepdims=True)
        p0 = jnp.exp(s0 - m0)
        init = (m0, jnp.sum(p0, axis=-1, keepdims=True),
                jnp.dot(p0.astype(_BF16), c0, preferred_element_type=_F32))

        def tile(i, carry):
            m, l, acc = carry
            wait_tile(i)

            @pl.when(i + KW < NT)
            def _():
                start_tile(i + KW)

            for k, cp in enumerate(c_wo):
                pl.when(i == NT - KW + k // WPI)(cp.start)
            tick(2 * i + j_loop)
            c = tile_ref(i)[...].reshape(T, DC)
            s = lax.dot_general(qa, c, _NT, preferred_element_type=_F32)
            m_new = jnp.maximum(m, jnp.max(s, axis=-1, keepdims=True))
            alpha = jnp.exp(m - m_new)
            p = jnp.exp(s - m_new)
            l = l * alpha + jnp.sum(p, axis=-1, keepdims=True)
            acc_v[...] = acc * alpha + jnp.dot(p.astype(_BF16), c,
                                               preferred_element_type=_F32)
            tick(2 * i + 1 + j_loop)
            return m_new, l, acc_v[...]

        _, l, acc = lax.fori_loop(0, NT, tile, init)

        ctx = contract((acc * (1.0 / l)).astype(_BF16).astype(_F32),
                       2).astype(_BF16).astype(_F32)
        for h in range(H - NV):
            lhs_v[:, h * D:(h + 1) * D] = jnp.broadcast_to(
                ctx[h:h + 1], (16, D)).astype(_BF16)
        for v in range(NV):
            cb_v[...] = jnp.broadcast_to(ctx[H - NV + v:H - NV + v + 1], (D, D))
            col_v[v * D:(v + 1) * D, :] = cb_v[...].T
        for j in range(j_loop + 2 * NT, NCH):
            tick(j)

        n_early = N1 + G1 // CH
        for j in range(NCH - RING, n_early):
            s2v(j).wait()
        g_v[...] = jnp.dot(h_v[:, 0:G1], w2_v[0:G1, :],
                           preferred_element_type=_F32)[0:8]

        for k, (a, b) in enumerate(zip(WO_SPLIT[:-1], WO_SPLIT[1:])):
            if k == 2:
                for j in range(max(n_early, NCH - RING), NCH):
                    s2v(j).wait()
                g = _silu(g_v[...] + jnp.dot(h_v[:, G1:F], w2_v[G1:F, :],
                                             preferred_element_type=_F32)[0:8])
                for bb in range(NB):
                    mult_v[:, bb * 128:(bb + 1) * 128] = (
                        col_v[...] * g[0:1, bb * 128:(bb + 1) * 128])
            c_wo[k].wait()
            if k < N_MXU:
                part = jnp.dot(lhs_v[:, a:b], wo_v[a:b, :],
                               preferred_element_type=_F32)[0:8]
                if k == 0:
                    s_v[...] = part
                elif k < N_MXU - 1:
                    s_v[...] += part
                else:
                    base = jnp.broadcast_to(x, (8, M)) + (s_v[...] + part) * g
                    row0 = lax.broadcasted_iota(jnp.int32, (8, M), 0) == 0
                    s_v[...] = jnp.where(row0, base, 0.0)
            else:
                r0 = a - (H - NV) * D
                prod = wo_v[a:b, :].astype(_F32) * mult_v[r0:r0 + b - a, :]
                parts = [s_v[...]] + [prod[r:r + 8] for r in range(0, b - a, 8)]
                while len(parts) > 1:
                    parts = [parts[i] + parts[i + 1] if i + 1 < len(parts)
                             else parts[i] for i in range(0, len(parts), 2)]
                if k < N_WO - 1:
                    s_v[...] = parts[0]
                else:
                    o_ref[0] = jnp.sum(parts[0], axis=0,
                                       keepdims=True).astype(o_ref.dtype)

    any_spec = pl.BlockSpec(memory_space=pl.ANY)
    return pl.pallas_call(
        kernel,
        out_shape=jax.ShapeDtypeStruct(A_x.shape, A_x.dtype),
        in_specs=[any_spec] * 8,
        out_specs=pl.BlockSpec(memory_space=pltpu.VMEM),
        scratch_shapes=[
            pltpu.VMEM(A_x.shape, _BF16),
            pltpu.VMEM((SM // KR, KR, DC), _BF16),
            pltpu.VMEM((KA, REM // KA, DC), _BF16),
            pltpu.VMEM((NB, LW, D), _BF16),
            pltpu.VMEM((NB, LW, D), _BF16),
            pltpu.VMEM((NB, LW, D), _BF16),
            pltpu.VMEM((H * D, M), _BF16),
            pltpu.VMEM((F, M), _BF16),
            pltpu.VMEM((F, M), _BF16),
            pltpu.VMEM((16, H * D), _BF16),
            pltpu.VMEM((8, M), _F32),
            pltpu.VMEM((8, M), _F32),
            pltpu.VMEM((16, F), _BF16),
            pltpu.VMEM((H, DC), _F32),
            pltpu.VMEM((D, D), _F32),
            pltpu.VMEM((D, D), _F32),
            pltpu.VMEM((NV * D, D), _F32),
            pltpu.VMEM((NV * D, M), _F32),
            pltpu.SMEM((RING, CH, M), _BF16),
            pltpu.SemaphoreType.DMA((3,)),
            pltpu.SemaphoreType.DMA((12,)),
            pltpu.SemaphoreType.DMA((NT,)),
            pltpu.SemaphoreType.DMA((N_WO,)),
            pltpu.SemaphoreType.DMA((RING,)),
            pltpu.SemaphoreType.DMA((RING,)),
        ],
        compiler_params=_compiler_params(),
    )(A_x, ckv2, wq2, wuk2, wuv2, wo2, w1t, B_w2)
```

```python
import functools

import jax
import jax.numpy as jnp
from jax import lax
import jax.experimental.pallas as pl
import jax.experimental.pallas.tpu as pltpu

_NT = (((1,), (1,)), ((), ()))
_F32 = jnp.float32
_BF16 = jnp.bfloat16


def _silu(v):
    return v * (1.0 / (1.0 + jnp.exp(-v)))


@jax.jit
def pallas_recurrent_scan__compressed_kv_cla__dense_activation_silu__decode_kernel(
    A_x: jax.Array,
    A_c_kv: jax.Array,
    A_w_q: jax.Array,
    A_w_uk: jax.Array,
    A_w_uv: jax.Array,
    A_w_o: jax.Array,
    B_x: jax.Array,
    B_w1: jax.Array,
    B_w2: jax.Array,
):
    del B_x
    B, Sq, M = A_x.shape
    _, S, DC = A_c_kv.shape
    _, H, D = A_w_q.shape
    F = B_w1.shape[1]
    assert (B, Sq, M, S, DC, H, D, F) == (1, 1, 512, 32768, 512, 32, 128, 1376)

    NB = 4
    G = 16
    NP = 128 // G

    KR, KA = 48, 4
    KQ = S // KA
    T = 1920
    NT = S // T
    SM = NT * T
    REM = S - SM
    DPT = T // (KA * KR)
    assert DPT * KA * KR == T
    KW = 2
    LW = 128 * H
    WR = 192
    WB = LW // WR
    GRP = (0, 5, 10, 15, WB)
    GW = 3

    CH, N1, AHEAD = 32, 6, 4
    RING = 2 * AHEAD
    NCH = N1 + F // CH
    R1 = N1 * CH
    G1 = 1152

    WO_SPLIT = (0, 16 * D, 24 * D, 28 * D, 30 * D, 31 * D,
                31 * D + 80, 31 * D + 112, 32 * D)
    N_WO = len(WO_SPLIT) - 1
    N_MXU = 4
    NV = H - WO_SPLIT[N_MXU] // D
    WPI = -(-N_WO // KW)

    ckv2 = A_c_kv.reshape(KA, KQ, DC)
    wq2 = A_w_q.reshape(NB, LW, D)
    wuk2 = A_w_uk.reshape(NB, LW, D)
    wuv2 = A_w_uv.reshape(NB, LW, D)
    wo2 = A_w_o.reshape(H * D, M)
    w1t = B_w1.T

    def kernel(*refs):
        pl.run_scoped(
            functools.partial(main, *refs),
            pltpu.SemaphoreType.DMA((3,)),
            pltpu.SemaphoreType.DMA((12,)),
            pltpu.SemaphoreType.DMA((NT,)),
            pltpu.SemaphoreType.DMA((N_WO,)),
            pltpu.SemaphoreType.DMA((RING,)),
            pltpu.SemaphoreType.DMA((RING,)),
        )

    def main(x_hbm, ckv_hbm, wq_hbm, wuk_hbm, wuv_hbm, wo_hbm, w1_hbm, w2_hbm,
             o_ref,
             x_v, ckv_v, rem_v, wq_v, wuk_v, wuv_v, wo_v, w1_v, w2_v,
             lhs_v, s_v, g_v, h_v, acc_v, cb_v, af_v, col_v, mult_v, stage,
             sems, g_sems, kv_sems, wo_sems, h2s_sems, s2v_sems):
        c_x = pltpu.make_async_copy(x_hbm, x_v, sems.at[0])
        c_w1 = pltpu.make_async_copy(w1_hbm.at[pl.ds(R1, F - R1)],
                                     w1_v.at[pl.ds(R1, F - R1)], sems.at[1])
        c_rem = pltpu.make_async_copy(
            ckv_hbm.at[:, pl.ds(SM // KA, REM // KA)], rem_v, sems.at[2])
        ws = [(wq_hbm, wq_v), (wuk_hbm, wuk_v), (wuv_hbm, wuv_v)]
        NG = 4 * len(ws)

        def start_group(g):
            src, dst = ws[g // 4]

            def body(b, carry):
                rows = pl.ds(pl.multiple_of(b * WR, WR), WR)
                pltpu.make_async_copy(src.at[:, rows], dst.at[:, rows],
                                      g_sems.at[g]).start()
                return carry

            lax.fori_loop(GRP[g % 4], GRP[g % 4 + 1], body, 0)
            if g % 4 == 3:
                rows = pl.ds(WB * WR, LW - WB * WR)
                pltpu.make_async_copy(src.at[:, rows], dst.at[:, rows],
                                      g_sems.at[g]).start()

        def wait_group(g):
            lo = GRP[g % 4] * WR
            hi = LW if g % 4 == 3 else GRP[g % 4 + 1] * WR
            region = ws[g // 4][1].at[:, pl.ds(lo, hi - lo)]
            pltpu.make_async_copy(region, region, g_sems.at[g]).wait()

        def start_tile(i):
            def body(dd, carry):
                d = i * DPT + dd
                pltpu.make_async_copy(
                    ckv_hbm.at[:, pl.ds(pl.multiple_of(d * KR, KR), KR)],
                    ckv_v.at[pl.ds(d * KA, KA)], kv_sems.at[i]).start()
                return carry

            lax.fori_loop(0, DPT, body, 0)

        def tile_ref(i):
            return ckv_v.at[pl.ds(i * (T // KR), T // KR)]

        def wait_tile(i):
            pltpu.make_async_copy(tile_ref(i), tile_ref(i),
                                  kv_sems.at[i]).wait()

        c_wo = [
            pltpu.make_async_copy(wo_hbm.at[pl.ds(a, b - a)],
                                  wo_v.at[pl.ds(a, b - a)], wo_sems.at[k])
            for k, (a, b) in enumerate(zip(WO_SPLIT[:-1], WO_SPLIT[1:]))
        ]

        def step(g):
            wait_group(g)
            if g + GW < NG:
                start_group(g + GW)
            elif g == NG - 3:
                c_rem.start()
                start_tile(0)
            elif g == NG - 1:
                start_tile(1)

        def chunk(j):
            if isinstance(j, int):
                if j < N1:
                    return w1_hbm, w1_v, pl.ds(j * CH, CH)
                return w2_hbm, w2_v, pl.ds((j - N1) * CH, CH)
            return w2_hbm, w2_v, pl.ds(pl.multiple_of((j - N1) * CH, CH), CH)

        def h2s(j):
            src, _, rows = chunk(j)
            slot = j % RING
            return pltpu.make_async_copy(
                src.at[rows], stage.at[slot], h2s_sems.at[slot])

        def s2v(j):
            _, dst, rows = chunk(j)
            slot = j % RING
            return pltpu.make_async_copy(
                stage.at[slot], dst.at[rows], s2v_sems.at[slot])

        def tick(j):
            h2s(j).wait()
            s2v(j).start()
            if isinstance(j, int):
                if j + AHEAD < NCH:
                    if j >= AHEAD:
                        s2v(j - AHEAD).wait()
                    h2s(j + AHEAD).start()
            else:
                @pl.when(j + AHEAD < NCH)
                def _():
                    s2v(j - AHEAD).wait()
                    h2s(j + AHEAD).start()

        def w_tiles(wi, n):
            w = ws[wi][1]
            return jnp.concatenate(
                [w[b, (n * G + jj) * H:(n * G + jj + 1) * H, :]
                 for jj in range(G) for b in range(NB)], axis=0)

        def head_mask(cols):
            r = lax.broadcasted_iota(jnp.int32, (H, cols), 0)
            c = lax.broadcasted_iota(jnp.int32, (H, cols), 1)
            return r == (c & (H - 1))

        def contract(a, wi):
            for b in range(NB):
                cb_v[b * H:(b + 1) * H, :] = a[:, b * 128:(b + 1) * 128]
            af_v[...] = cb_v[...].T
            mask = head_mask(128)
            out = jnp.zeros((H, D), _F32)
            for n in range(NP):
                lhs = jnp.concatenate(
                    [jnp.where(mask, af_v[pl.ds(n * G + jj, 1), :], 0.0)
                     .astype(_BF16) for jj in range(G)], axis=1)
                out = out + jnp.dot(lhs, w_tiles(wi, n),
                                    preferred_element_type=_F32)
            return out

        c_w1.start()
        h2s(0).start()
        start_group(0)
        for j in range(1, AHEAD):
            h2s(j).start()
        c_x.start()
        for g in range(1, GW):
            start_group(g)
        tick(0)
        c_w1.wait()
        tick(1)
        for g in range(8):
            step(g)
            tick(g + 2)

        c_x.wait()
        x = x_v[0].astype(_F32)
        mu = jnp.mean(x, axis=-1, keepdims=True)
        xc = x - mu
        var = jnp.mean(xc * xc, axis=-1, keepdims=True)
        xn = xc * lax.rsqrt(var + 1e-5)
        lhs_v[:, 0:M] = jnp.broadcast_to(xn, (16, M)).astype(_BF16)
        xn16 = lhs_v[:, 0:M]
        q = contract(jnp.concatenate([xn16, xn16], axis=0).astype(_F32),
                     0).astype(_BF16)
        step(8)
        tick(10)

        for n in range(NP):
            t = lax.dot_general(q, w_tiles(1, n), _NT,
                                preferred_element_type=_F32)
            r = jnp.sum(jnp.where(head_mask(G * 128), t, 0.0), axis=0,
                        keepdims=True)
            for jj in range(G):
                af_v[pl.ds(n * G + jj, 1), :] = r[:, jj * 128:(jj + 1) * 128]
            if n == NP // 2 - 1:
                step(9)
                tick(11)
        z = af_v[...].T * (D ** -0.5)
        qa = jnp.concatenate(
            [z[b * H:(b + 1) * H] for b in range(NB)], axis=1).astype(_BF16)
        step(10)
        tick(12)
        step(11)
        tick(13)
        j_loop = 14
        assert j_loop - AHEAD >= N1 and j_loop + 2 * NT <= NCH

        h1 = lax.dot_general(xn16, w1_v[...], _NT, preferred_element_type=_F32)
        h_v[...] = _silu(h1).astype(_BF16)

        c_rem.wait()
        c0 = rem_v[...].reshape(REM, DC)
        s0 = lax.dot_general(qa, c0, _NT, preferred_element_type=_F32)
        m0 = jnp.max(s0, axis=-1, keepdims=True)
        p0 = jnp.exp(s0 - m0)
        init = (m0, jnp.sum(p0, axis=-1, keepdims=True),
                jnp.dot(p0.astype(_BF16), c0, preferred_element_type=_F32))

        def tile(i, carry):
            m, l, acc = carry
            wait_tile(i)

            @pl.when(i + KW < NT)
            def _():
                start_tile(i + KW)

            for k, cp in enumerate(c_wo):
                pl.when(i == NT - KW + k // WPI)(cp.start)
            tick(2 * i + j_loop)
            c = tile_ref(i)[...].reshape(T, DC)
            s = lax.dot_general(qa, c, _NT, preferred_element_type=_F32)
            m_new = jnp.maximum(m, jnp.max(s, axis=-1, keepdims=True))
            alpha = jnp.exp(m - m_new)
            p = jnp.exp(s - m_new)
            l = l * alpha + jnp.sum(p, axis=-1, keepdims=True)
            acc_v[...] = acc * alpha + jnp.dot(p.astype(_BF16), c,
                                               preferred_element_type=_F32)
            tick(2 * i + 1 + j_loop)
            return m_new, l, acc_v[...]

        _, l, acc = lax.fori_loop(0, NT, tile, init)

        ctx = contract((acc * (1.0 / l)).astype(_BF16).astype(_F32),
                       2).astype(_BF16).astype(_F32)
        for h in range(H - NV):
            lhs_v[:, h * D:(h + 1) * D] = jnp.broadcast_to(
                ctx[h:h + 1], (16, D)).astype(_BF16)
        for v in range(NV):
            cb_v[...] = jnp.broadcast_to(ctx[H - NV + v:H - NV + v + 1], (D, D))
            col_v[v * D:(v + 1) * D, :] = cb_v[...].T
        for j in range(j_loop + 2 * NT, NCH):
            tick(j)

        n_early = N1 + G1 // CH
        for j in range(NCH - RING, n_early):
            s2v(j).wait()
        g_v[...] = jnp.dot(h_v[:, 0:G1], w2_v[0:G1, :],
                           preferred_element_type=_F32)[0:8]

        for k, (a, b) in enumerate(zip(WO_SPLIT[:-1], WO_SPLIT[1:])):
            if k == 2:
                for j in range(max(n_early, NCH - RING), NCH):
                    s2v(j).wait()
                g = _silu(g_v[...] + jnp.dot(h_v[:, G1:F], w2_v[G1:F, :],
                                             preferred_element_type=_F32)[0:8])
                for bb in range(NB):
                    mult_v[:, bb * 128:(bb + 1) * 128] = (
                        col_v[...] * g[0:1, bb * 128:(bb + 1) * 128])
            c_wo[k].wait()
            if k < N_MXU:
                part = jnp.dot(lhs_v[:, a:b], wo_v[a:b, :],
                               preferred_element_type=_F32)[0:8]
                if k == 0:
                    s_v[...] = part
                elif k < N_MXU - 1:
                    s_v[...] += part
                else:
                    base = jnp.broadcast_to(x, (8, M)) + (s_v[...] + part) * g
                    row0 = lax.broadcasted_iota(jnp.int32, (8, M), 0) == 0
                    s_v[...] = jnp.where(row0, base, 0.0)
            else:
                r0 = a - (H - NV) * D
                prod = wo_v[a:b, :].astype(_F32) * mult_v[r0:r0 + b - a, :]
                parts = [s_v[...]] + [prod[r:r + 8] for r in range(0, b - a, 8)]
                while len(parts) > 1:
                    parts = [parts[i] + parts[i + 1] if i + 1 < len(parts)
                             else parts[i] for i in range(0, len(parts), 2)]
                if k < N_WO - 1:
                    s_v[...] = parts[0]
                else:
                    o_ref[0] = jnp.sum(parts[0], axis=0,
                                       keepdims=True).astype(o_ref.dtype)

    any_spec = pl.BlockSpec(memory_space=pl.ANY)
    return pl.pallas_call(
        kernel,
        out_shape=jax.ShapeDtypeStruct(A_x.shape, A_x.dtype),
        in_specs=[any_spec] * 8,
        out_specs=pl.BlockSpec(memory_space=pltpu.VMEM),
        scratch_shapes=[
            pltpu.VMEM(A_x.shape, _BF16),
            pltpu.VMEM((SM // KR, KR, DC), _BF16),
            pltpu.VMEM((KA, REM // KA, DC), _BF16),
            pltpu.VMEM((NB, LW, D), _BF16),
            pltpu.VMEM((NB, LW, D), _BF16),
            pltpu.VMEM((NB, LW, D), _BF16),
            pltpu.VMEM((H * D, M), _BF16),
            pltpu.VMEM((F, M), _BF16),
            pltpu.VMEM((F, M), _BF16),
            pltpu.VMEM((16, H * D), _BF16),
            pltpu.VMEM((8, M), _F32),
            pltpu.VMEM((8, M), _F32),
            pltpu.VMEM((16, F), _BF16),
            pltpu.VMEM((H, DC), _F32),
            pltpu.VMEM((D, D), _F32),
            pltpu.VMEM((D, D), _F32),
            pltpu.VMEM((NV * D, D), _F32),
            pltpu.VMEM((NV * D, M), _F32),
            pltpu.SMEM((RING, CH, M), _BF16),
        ],
        compiler_params=pltpu.CompilerParams(
            vmem_limit_bytes=100 * 1024 * 1024),
    )(A_x, ckv2, wq2, wuk2, wuv2, wo2, w1t, B_w2)
```

```python
import functools

import jax
import jax.numpy as jnp
from jax import lax
import jax.experimental.pallas as pl
import jax.experimental.pallas.tpu as pltpu

_NT = (((1,), (1,)), ((), ()))
_F32 = jnp.float32
_BF16 = jnp.bfloat16


def _silu(v):
    return v * (1.0 / (1.0 + jnp.exp(-v)))


@jax.jit
def pallas_recurrent_scan__compressed_kv_cla__dense_activation_silu__decode_kernel(
    A_x: jax.Array,
    A_c_kv: jax.Array,
    A_w_q: jax.Array,
    A_w_uk: jax.Array,
    A_w_uv: jax.Array,
    A_w_o: jax.Array,
    B_x: jax.Array,
    B_w1: jax.Array,
    B_w2: jax.Array,
):
    del B_x
    B, Sq, M = A_x.shape
    _, S, DC = A_c_kv.shape
    _, H, D = A_w_q.shape
    F = B_w1.shape[1]
    assert (B, Sq, M, S, DC, H, D, F) == (1, 1, 512, 32768, 512, 32, 128, 1376)

    NB = 4
    G = 16
    NP = 128 // G

    KR, KA, KV = 48, 4, 8
    KQ = S // KV
    KB = KQ // KR
    T = 1920
    NT = S // T
    SM = NT * T
    REM = S - SM
    DPT = T // (KA * KR)
    assert DPT * KA * KR == T and KV * KB * KR == SM
    KW = 2
    LW = 128 * H
    WR = 192
    WB = LW // WR
    GRP = (0, 5, 10, 15, WB)
    GW = 3

    CH, N1, AHEAD = 32, 6, 4
    RING = 2 * AHEAD
    NCH = N1 + F // CH
    R1 = N1 * CH
    G1 = 1152

    WO_SPLIT = (0, 16 * D, 24 * D, 28 * D, 30 * D, 31 * D,
                31 * D + 80, 31 * D + 112, 32 * D)
    N_WO = len(WO_SPLIT) - 1
    N_MXU = 4
    NV = H - WO_SPLIT[N_MXU] // D
    WPI = -(-N_WO // KW)

    ckv2 = A_c_kv.reshape(KV, KQ, DC)
    wq2 = A_w_q.reshape(NB, LW, D)
    wuk2 = A_w_uk.reshape(NB, LW, D)
    wuv2 = A_w_uv.reshape(NB, LW, D)
    wo2 = A_w_o.reshape(H * D, M)
    w1t = B_w1.T

    def kernel(*refs):
        pl.run_scoped(
            functools.partial(main, *refs),
            pltpu.SemaphoreType.DMA((3,)),
            pltpu.SemaphoreType.DMA((12,)),
            pltpu.SemaphoreType.DMA((NT,)),
            pltpu.SemaphoreType.DMA((N_WO,)),
            pltpu.SemaphoreType.DMA((RING,)),
            pltpu.SemaphoreType.DMA((RING,)),
        )

    def main(x_hbm, ckv_hbm, wq_hbm, wuk_hbm, wuv_hbm, wo_hbm, w1_hbm, w2_hbm,
             o_ref,
             x_v, ckv_v, rem_v, wq_v, wuk_v, wuv_v, wo_v, w1_v, w2_v,
             lhs_v, s_v, g_v, h_v, acc_v, cb_v, af_v, col_v, mult_v, stage,
             sems, g_sems, kv_sems, wo_sems, h2s_sems, s2v_sems):
        c_x = pltpu.make_async_copy(x_hbm, x_v, sems.at[0])
        c_w1 = pltpu.make_async_copy(w1_hbm.at[pl.ds(R1, F - R1)],
                                     w1_v.at[pl.ds(R1, F - R1)], sems.at[1])
        c_rem = pltpu.make_async_copy(
            ckv_hbm.at[:, pl.ds(KB * KR, REM // KV)], rem_v, sems.at[2])
        ws = [(wq_hbm, wq_v), (wuk_hbm, wuk_v), (wuv_hbm, wuv_v)]
        NG = 4 * len(ws)

        def start_group(g):
            src, dst = ws[g // 4]

            def body(b, carry):
                rows = pl.ds(pl.multiple_of(b * WR, WR), WR)
                pltpu.make_async_copy(src.at[:, rows], dst.at[:, rows],
                                      g_sems.at[g]).start()
                return carry

            lax.fori_loop(GRP[g % 4], GRP[g % 4 + 1], body, 0)
            if g % 4 == 3:
                rows = pl.ds(WB * WR, LW - WB * WR)
                pltpu.make_async_copy(src.at[:, rows], dst.at[:, rows],
                                      g_sems.at[g]).start()

        def wait_group(g):
            lo = GRP[g % 4] * WR
            hi = LW if g % 4 == 3 else GRP[g % 4 + 1] * WR
            region = ws[g // 4][1].at[:, pl.ds(lo, hi - lo)]
            pltpu.make_async_copy(region, region, g_sems.at[g]).wait()

        def start_tile(i):
            def body(dd, carry):
                d = i * DPT + dd
                blocks = pl.ds((d // KB) * KA, KA)
                rows = pl.ds(pl.multiple_of((d % KB) * KR, KR), KR)
                pltpu.make_async_copy(
                    ckv_hbm.at[blocks, rows], ckv_v.at[pl.ds(d * KA, KA)],
                    kv_sems.at[i]).start()
                return carry

            lax.fori_loop(0, DPT, body, 0)

        def tile_ref(i):
            return ckv_v.at[pl.ds(i * (T // KR), T // KR)]

        def wait_tile(i):
            pltpu.make_async_copy(tile_ref(i), tile_ref(i),
                                  kv_sems.at[i]).wait()

        c_wo = [
            pltpu.make_async_copy(wo_hbm.at[pl.ds(a, b - a)],
                                  wo_v.at[pl.ds(a, b - a)], wo_sems.at[k])
            for k, (a, b) in enumerate(zip(WO_SPLIT[:-1], WO_SPLIT[1:]))
        ]

        def step(g):
            wait_group(g)
            if g + GW < NG:
                start_group(g + GW)
            elif g == NG - 3:
                c_rem.start()
                start_tile(0)
            elif g == NG - 1:
                start_tile(1)

        def chunk(j):
            if isinstance(j, int):
                if j < N1:
                    return w1_hbm, w1_v, pl.ds(j * CH, CH)
                return w2_hbm, w2_v, pl.ds((j - N1) * CH, CH)
            return w2_hbm, w2_v, pl.ds(pl.multiple_of((j - N1) * CH, CH), CH)

        def h2s(j):
            src, _, rows = chunk(j)
            slot = j % RING
            return pltpu.make_async_copy(
                src.at[rows], stage.at[slot], h2s_sems.at[slot])

        def s2v(j):
            _, dst, rows = chunk(j)
            slot = j % RING
            return pltpu.make_async_copy(
                stage.at[slot], dst.at[rows], s2v_sems.at[slot])

        def tick(j):
            h2s(j).wait()
            s2v(j).start()
            if isinstance(j, int):
                if j + AHEAD < NCH:
                    if j >= AHEAD:
                        s2v(j - AHEAD).wait()
                    h2s(j + AHEAD).start()
            else:
                @pl.when(j + AHEAD < NCH)
                def _():
                    s2v(j - AHEAD).wait()
                    h2s(j + AHEAD).start()

        def w_tiles(wi, n):
            w = ws[wi][1]
            return jnp.concatenate(
                [w[b, (n * G + jj) * H:(n * G + jj + 1) * H, :]
                 for jj in range(G) for b in range(NB)], axis=0)

        def head_mask(cols):
            r = lax.broadcasted_iota(jnp.int32, (H, cols), 0)
            c = lax.broadcasted_iota(jnp.int32, (H, cols), 1)
            return r == (c & (H - 1))

        def contract(a, wi):
            for b in range(NB):
                cb_v[b * H:(b + 1) * H, :] = a[:, b * 128:(b + 1) * 128]
            af_v[...] = cb_v[...].T
            mask = head_mask(128)
            out = jnp.zeros((H, D), _F32)
            for n in range(NP):
                lhs = jnp.concatenate(
                    [jnp.where(mask, af_v[pl.ds(n * G + jj, 1), :], 0.0)
                     .astype(_BF16) for jj in range(G)], axis=1)
                out = out + jnp.dot(lhs, w_tiles(wi, n),
                                    preferred_element_type=_F32)
            return out

        c_w1.start()
        h2s(0).start()
        start_group(0)
        for j in range(1, AHEAD):
            h2s(j).start()
        c_x.start()
        for g in range(1, GW):
            start_group(g)
        tick(0)
        c_w1.wait()
        tick(1)
        for g in range(8):
            step(g)
            tick(g + 2)

        c_x.wait()
        x = x_v[0].astype(_F32)
        mu = jnp.mean(x, axis=-1, keepdims=True)
        xc = x - mu
        var = jnp.mean(xc * xc, axis=-1, keepdims=True)
        xn = xc * lax.rsqrt(var + 1e-5)
        lhs_v[:, 0:M] = jnp.broadcast_to(xn, (16, M)).astype(_BF16)
        xn16 = lhs_v[:, 0:M]
        q = contract(jnp.concatenate([xn16, xn16], axis=0).astype(_F32),
                     0).astype(_BF16)
        step(8)
        tick(10)

        for n in range(NP):
            t = lax.dot_general(q, w_tiles(1, n), _NT,
                                preferred_element_type=_F32)
            r = jnp.sum(jnp.where(head_mask(G * 128), t, 0.0), axis=0,
                        keepdims=True)
            for jj in range(G):
                af_v[pl.ds(n * G + jj, 1), :] = r[:, jj * 128:(jj + 1) * 128]
            if n == NP // 2 - 1:
                step(9)
                tick(11)
        z = af_v[...].T * (D ** -0.5)
        qa = jnp.concatenate(
            [z[b * H:(b + 1) * H] for b in range(NB)], axis=1).astype(_BF16)
        step(10)
        tick(12)
        step(11)
        tick(13)
        j_loop = 14
        assert j_loop - AHEAD >= N1 and j_loop + 2 * NT <= NCH

        h1 = lax.dot_general(xn16, w1_v[...], _NT, preferred_element_type=_F32)
        h_v[...] = _silu(h1).astype(_BF16)

        c_rem.wait()
        c0 = rem_v[...].reshape(REM, DC)
        s0 = lax.dot_general(qa, c0, _NT, preferred_element_type=_F32)
        m0 = jnp.max(s0, axis=-1, keepdims=True)
        p0 = jnp.exp(s0 - m0)
        init = (m0, jnp.sum(p0, axis=-1, keepdims=True),
                jnp.dot(p0.astype(_BF16), c0, preferred_element_type=_F32))

        def tile(i, carry):
            m, l, acc = carry
            wait_tile(i)

            @pl.when(i + KW < NT)
            def _():
                start_tile(i + KW)

            for k, cp in enumerate(c_wo):
                pl.when(i == NT - KW + k // WPI)(cp.start)
            tick(2 * i + j_loop)
            c = tile_ref(i)[...].reshape(T, DC)
            s = lax.dot_general(qa, c, _NT, preferred_element_type=_F32)
            m_new = jnp.maximum(m, jnp.max(s, axis=-1, keepdims=True))
            alpha = jnp.exp(m - m_new)
            p = jnp.exp(s - m_new)
            l = l * alpha + jnp.sum(p, axis=-1, keepdims=True)
            acc_v[...] = acc * alpha + jnp.dot(p.astype(_BF16), c,
                                               preferred_element_type=_F32)
            tick(2 * i + 1 + j_loop)
            return m_new, l, acc_v[...]

        _, l, acc = lax.fori_loop(0, NT, tile, init)

        ctx = contract((acc * (1.0 / l)).astype(_BF16).astype(_F32),
                       2).astype(_BF16).astype(_F32)
        for h in range(H - NV):
            lhs_v[:, h * D:(h + 1) * D] = jnp.broadcast_to(
                ctx[h:h + 1], (16, D)).astype(_BF16)
        for v in range(NV):
            cb_v[...] = jnp.broadcast_to(ctx[H - NV + v:H - NV + v + 1], (D, D))
            col_v[v * D:(v + 1) * D, :] = cb_v[...].T
        for j in range(j_loop + 2 * NT, NCH):
            tick(j)

        n_early = N1 + G1 // CH
        for j in range(NCH - RING, n_early):
            s2v(j).wait()
        g_v[...] = jnp.dot(h_v[:, 0:G1], w2_v[0:G1, :],
                           preferred_element_type=_F32)[0:8]

        for k, (a, b) in enumerate(zip(WO_SPLIT[:-1], WO_SPLIT[1:])):
            if k == 2:
                for j in range(max(n_early, NCH - RING), NCH):
                    s2v(j).wait()
                g = _silu(g_v[...] + jnp.dot(h_v[:, G1:F], w2_v[G1:F, :],
                                             preferred_element_type=_F32)[0:8])
                for bb in range(NB):
                    mult_v[:, bb * 128:(bb + 1) * 128] = (
                        col_v[...] * g[0:1, bb * 128:(bb + 1) * 128])
            c_wo[k].wait()
            if k < N_MXU:
                part = jnp.dot(lhs_v[:, a:b], wo_v[a:b, :],
                               preferred_element_type=_F32)[0:8]
                if k == 0:
                    s_v[...] = part
                elif k < N_MXU - 1:
                    s_v[...] += part
                else:
                    base = jnp.broadcast_to(x, (8, M)) + (s_v[...] + part) * g
                    row0 = lax.broadcasted_iota(jnp.int32, (8, M), 0) == 0
                    s_v[...] = jnp.where(row0, base, 0.0)
            else:
                r0 = a - (H - NV) * D
                prod = wo_v[a:b, :].astype(_F32) * mult_v[r0:r0 + b - a, :]
                parts = [s_v[...]] + [prod[r:r + 8] for r in range(0, b - a, 8)]
                while len(parts) > 1:
                    parts = [parts[i] + parts[i + 1] if i + 1 < len(parts)
                             else parts[i] for i in range(0, len(parts), 2)]
                if k < N_WO - 1:
                    s_v[...] = parts[0]
                else:
                    o_ref[0] = jnp.sum(parts[0], axis=0,
                                       keepdims=True).astype(o_ref.dtype)

    any_spec = pl.BlockSpec(memory_space=pl.ANY)
    return pl.pallas_call(
        kernel,
        out_shape=jax.ShapeDtypeStruct(A_x.shape, A_x.dtype),
        in_specs=[any_spec] * 8,
        out_specs=pl.BlockSpec(memory_space=pltpu.VMEM),
        scratch_shapes=[
            pltpu.VMEM(A_x.shape, _BF16),
            pltpu.VMEM((SM // KR, KR, DC), _BF16),
            pltpu.VMEM((KV, REM // KV, DC), _BF16),
            pltpu.VMEM((NB, LW, D), _BF16),
            pltpu.VMEM((NB, LW, D), _BF16),
            pltpu.VMEM((NB, LW, D), _BF16),
            pltpu.VMEM((H * D, M), _BF16),
            pltpu.VMEM((F, M), _BF16),
            pltpu.VMEM((F, M), _BF16),
            pltpu.VMEM((16, H * D), _BF16),
            pltpu.VMEM((8, M), _F32),
            pltpu.VMEM((8, M), _F32),
            pltpu.VMEM((16, F), _BF16),
            pltpu.VMEM((H, DC), _F32),
            pltpu.VMEM((D, D), _F32),
            pltpu.VMEM((D, D), _F32),
            pltpu.VMEM((NV * D, D), _F32),
            pltpu.VMEM((NV * D, M), _F32),
            pltpu.SMEM((RING, CH, M), _BF16),
        ],
        compiler_params=pltpu.CompilerParams(
            vmem_limit_bytes=100 * 1024 * 1024),
    )(A_x, ckv2, wq2, wuk2, wuv2, wo2, w1t, B_w2)
```
